```python
import os as _os
_os.environ.setdefault("JAX_PLATFORMS", "cpu")
import jax
import jax.numpy as jnp

def _softmax(x, axis=-1):
    return jax.nn.softmax(x, axis=axis)
def _gelu(x):
    return jax.nn.gelu(x, approximate=True)
def _silu(x):
    return jax.nn.silu(x)
def _sigmoid(x):
    return jax.nn.sigmoid(x)
def _layernorm(x, axis=-1, eps=1e-5):
    m = jnp.mean(x, axis=axis, keepdims=True)
    v = jnp.var(x, axis=axis, keepdims=True)
    return (x - m) / jnp.sqrt(v + eps)
def _scatter_add(tgt, idx, src, axis=0):
    return tgt.at[idx].add(src)
def _segment_sum(src, seg, n):
    return jax.ops.segment_sum(src, seg, n)
class _Rng:
    def __init__(self, key):
        self._k = key
    def _next(self):
        self._k, sub = jax.random.split(self._k)
        return sub
    def normal(self, shape):
        return jax.random.normal(self._next(), shape, dtype=jnp.bfloat16)
    def randint(self, lo, hi, shape):
        return jax.random.randint(self._next(), shape, lo, hi, dtype=jnp.int32)
    def uniform(self, shape, lo=0.0, hi=1.0):
        return jax.random.uniform(self._next(), shape, jnp.bfloat16, lo, hi)
    def permutation(self, n):
        return jax.random.permutation(self._next(), n)


kernel_name = 'sequential_preLN__ssm_conv_h3__dense_activation_gelu__prompt'

def setup_inputs():
    _rng = _Rng(jax.random.key(int.from_bytes(__import__("os").urandom(4), "little")))
    _w = (lambda a: (lambda t: t.astype(jnp.bfloat16) if jnp.issubdtype(t.dtype, jnp.floating) else t)(jnp.asarray(a)))
    def _A_setup():
        B, S, D = 1, 2048, 512
        ks = 4
        return {
            "q": _w((lambda *s: _rng.normal(s) * 0.05)(B, S, D)),
            "k": _w((lambda *s: _rng.normal(s) * 0.2)(B, S, D)),
            "v": _w((lambda *s: _rng.normal(s) * 0.2)(B, S, D)),
            "shift_k": _w((lambda *s: _rng.normal(s) * 0.2)(D, ks) * 0.5),
            "ssm_k": _w((lambda *s: _rng.normal(s) * 0.2)(D, S) * (1.0 / S ** 0.5)),
            "ssm_D": _w((lambda *s: _rng.normal(s) * 0.2)(D)),
        }
    _A_in = _A_setup()

    def _B_setup():
        B, S, D, F = 1, 2048, 512, 1376
        return {
            "x": _w((lambda *s: _rng.normal(s) * 0.05)(B, S, D)),
            "w1": _w((lambda *s: _rng.normal(s) * 0.2)(D, F) * (D ** -0.5)),
            "b1": _w((lambda *s: _rng.normal(s) * 0.2)(F) * 0.01),
            "w2": _w((lambda *s: _rng.normal(s) * 0.2)(F, D) * (F ** -0.5)),
            "b2": _w((lambda *s: _rng.normal(s) * 0.05)(D) * 0.01),
        }
    _B_in = _B_setup()

    return {
        "A_q": _A_in["q"],
        "A_k": _A_in["k"],
        "A_v": _A_in["v"],
        "A_shift_k": _A_in["shift_k"],
        "A_ssm_k": _A_in["ssm_k"],
        "A_ssm_D": _A_in["ssm_D"],
        "B_x": _B_in["x"],
        "B_w1": _B_in["w1"],
        "B_b1": _B_in["b1"],
        "B_w2": _B_in["w2"],
        "B_b2": _B_in["b2"],
    }

def reference(A_q, A_k, A_v, A_shift_k, A_ssm_k, A_ssm_D, B_x, B_w1, B_b1, B_w2, B_b2):
    def _A_ref(q, k, v, shift_k, ssm_k, ssm_D):
        B, S, D = q.shape
        ks = shift_k.shape[-1]
        k_pad = jnp.pad(k, ((0, 0), (ks - 1, 0), (0, 0)))
        k_shift = jnp.zeros_like(k)
        for t in range(ks):
            k_shift = k_shift + k_pad[:, t:t + S, :] * shift_k[:, ks - 1 - t][None, None, :]
        kv = k_shift * v
        L = 2 * S
        kv_pad = jnp.pad(kv, ((0, 0), (0, S), (0, 0)))
        kf_pad = jnp.pad(ssm_k, ((0, 0), (0, S)))
        kv_f = (lambda x, axes=(-2,-1): jnp.fft.rfft2(x.astype(jnp.float32), axes=axes))(kv_pad[:, None, :, :], axes=(1, 2))
        kf_f = (lambda x, axes=(-2,-1): jnp.fft.rfft2(x.astype(jnp.float32), axes=axes))(kf_pad[:, None, :], axes=(1, 2))
        kf_f = (lambda x, *d: x.transpose(*d))(kf_f, 1, 2, 0)
        y_f = kv_f * kf_f[None, :, :, :]
        y = (lambda x, s, axes=(-2,-1): jnp.fft.irfft2(x, s=s, axes=axes).astype(jnp.bfloat16))(y_f, (1, L), axes=(1, 2))[:, 0, :S, :]
        y = y + kv * ssm_D[None, None, :]
        return q * y

    def _B_ref(x, w1, b1, w2, b2):
        h = jnp.einsum("bsd,df->bsf", x, w1) + b1
        h = _gelu(h)
        return jnp.einsum("bsf,fd->bsd", h, w2) + b2

    x = A_q
    h = x + _A_ref(_layernorm(x, axis=-1), A_k, A_v, A_shift_k, A_ssm_k, A_ssm_D)
    h2 = h + _B_ref(_layernorm(h, axis=-1), B_w1, B_b1, B_w2, B_b2)
    return h2
```

```python
import functools
import math

import jax
import jax.numpy as jnp
from jax import lax
import jax.experimental.pallas as pl
import jax.experimental.pallas.tpu as pltpu

S, D, F = 2048, 512, 1376
B = 128
NB = S // B
NL = D // 128
NF = (F + 127) // 128
EPS = 1e-5
f32, bf16, u32 = jnp.float32, jnp.bfloat16, jnp.uint32
NT = (((1,), (1,)), ((), ()))
C0 = math.sqrt(2.0 / math.pi)
C1 = C0 * 0.044715
KG = ((0, 512), (512, 1024), (1024, F))


def _kernel(q_hbm, k_hbm, v_hbm, sk_hbm, ssm_hbm, sd_hbm, w1t_hbm, b1_hbm, w2_hbm, b2_hbm,
            o_hbm,
            qb, kb, vb, ssm, w1t, w2, skb, sdb, b1b, b2b, kf, ob,
            w1u, w2u, fu, gu, XS, KS, PS, KV, HR, YS, HN, H1,
            isem, osem, zsem, *, plan):
    cfg = plan["cfg"]
    zero = pl.semaphore_read(zsem.at[0])

    sem_id = [0]

    def cp(src, dst):
        c = pltpu.make_async_copy(src, dst, isem.at[sem_id[0]])
        sem_id[0] += 1
        return c

    def blk_copies(b0, b1):
        r = pl.ds(b0 * B, (b1 - b0) * B)
        return [cp(k_hbm.at[r], kb.at[r]), cp(v_hbm.at[r], vb.at[r]),
                cp(ssm_hbm.at[:, r], ssm.at[:, r]), cp(q_hbm.at[r], qb.at[r])]

    groups = {}
    for name, spec in plan["dma"]:
        cs = []
        for item in spec:
            if item == "small":
                cs += [cp(sk_hbm, skb), cp(sd_hbm, sdb), cp(b1_hbm, b1b), cp(b2_hbm, b2b)]
            elif item == "w1":
                cs += [cp(w1t_hbm, w1t)]
            elif item == "w2":
                cs += [cp(w2_hbm, w2)]
            else:
                r = pl.ds(item[1] * B, (item[2] - item[1]) * B)
                for ch in item[0]:
                    if ch == "s":
                        cs.append(cp(ssm_hbm.at[:, r], ssm.at[:, r]))
                    else:
                        src, dst = dict(k=(k_hbm, kb), v=(v_hbm, vb), q=(q_hbm, qb))[ch]
                        cs.append(cp(src.at[r], dst.at[r]))
        groups[name] = cs
        for c in cs:
            c.start()
    out_copies = [pltpu.make_async_copy(ob.at[pl.ds(b * B, B)], o_hbm.at[pl.ds(b * B, B)], osem.at[b])
                  for b in range(NB)]

    Q = dict(post=[], c=[], kv=[], mac=[])
    st = dict(credit=0.0, never=None, cache={}, macrate=1e9, maccredit=0.0)

    def cached(key, fn):
        if key not in st["cache"]:
            st["cache"][key] = fn()
        return st["cache"][key]

    def LT(l):
        return slice(l * 128, (l + 1) * 128)

    def tables():
        def cosn(r, j, scale):
            rr = r & (B - 1)
            odd = 4 * rr + jnp.where(rr < B // 2, 1, 3 - 2 * B)
            n = (odd * j + (r & B)) & (4 * B - 1)
            n = jnp.abs(n - 2 * B)
            m = B - n
            x = m.astype(f32) * (-2.0 * math.pi / (4 * B))
            x2 = x * x
            p = -1.0 / 39916800.0
            for cf in (1.0 / 362880.0, -1.0 / 5040.0, 1.0 / 120.0, -1.0 / 6.0, 1.0):
                p = p * x2 + cf
            return p * (x * scale)

        r = lax.broadcasted_iota(jnp.int32, (2 * B, B), 0)
        r = ((r >> 5) << 4) + (r & 15) + ((r & 16) << 3)
        j = lax.broadcasted_iota(jnp.int32, (2 * B, B), 1)
        fu[...] = pltpu.bitcast(cosn(r, j, 1.0).astype(bf16), u32)
        r = lax.broadcasted_iota(jnp.int32, (B, 2 * B), 1)
        j = lax.broadcasted_iota(jnp.int32, (B, 2 * B), 0)
        gu[...] = pltpu.bitcast(cosn(r, j, 1.0 / B).astype(bf16), u32)
        for l in range(NL):
            kf[l, 0:8, :] = jnp.zeros((8, 128), f32)

    kvv = {}
    ymark = {}

    def kv_job(b, g):
        r0 = b * B + 8 * g
        sk = cached("sk", lambda: skb[...].astype(f32))
        kall = kb[r0:r0 + 8, :].astype(f32)
        vall = vb[r0:r0 + 8, :].astype(f32)
        outs = []
        for l in range(NL):
            kk = kall[:, LT(l)]
            kf[l, 8 + r0:16 + r0, :] = kk
            acc = kk * sk[0:1, LT(l)]
            for t in range(1, 4):
                acc = acc + kf[l, 8 + r0 - t:16 + r0 - t, :] * sk[t:t + 1, LT(l)]
            outs.append(acc * vall[:, LT(l)])
        kv = jnp.concatenate(outs, axis=1)
        KV[r0:r0 + 8, :] = kv
        kvv.setdefault(b, []).append(kv)
        return outs

    def push_kv(b):
        for g in range(16):
            Q["kv"].append([0, 44, functools.partial(kv_job, b, g)])

    ready = set()

    def split_ri(h, g):
        r0 = (g // 2) * 32 + (g % 2) * 8
        return h[r0:r0 + 8], h[r0 + 16:r0 + 24]

    def stage_x(b):
        while Q["kv"] and len(kvv.get(b, [])) < 16:
            Q["kv"].pop(0)[2]()
        kv = jnp.concatenate(kvv.pop(b), axis=0)
        fm = pltpu.bitcast(fu[...], bf16)
        xh = jnp.dot(fm, kv.astype(bf16), preferred_element_type=f32)
        for g in range(16):
            a, bb = split_ri(xh, g)
            R = slice(8 * g, 8 * g + 8)
            XS[b, 1, R, :] = a
            XS[b, 2, R, :] = bb
            a = jnp.concatenate([slot(a[:, LT(l)], cfg["capx"] * 4, 4) for l in range(NL)], axis=1)
            XS[b, 0, R, :] = a + bb
        ready.add(("x", b))

    def stage_k(a):
        fm = pltpu.bitcast(fu[...], bf16)
        kh = lax.dot_general(fm, ssm[:, a * B:(a + 1) * B], NT, preferred_element_type=f32)
        for g in range(16):
            c, d = split_ri(kh, g)
            R = slice(8 * g, 8 * g + 8)
            KS[a, 0, R, :] = c
            c = jnp.concatenate([slot(c[:, LT(l)], cfg["capx"] * 4, 4) for l in range(NL)], axis=1)
            KS[a, 1, R, :] = d - c
            KS[a, 2, R, :] = c + d
        ready.add(("k", a))

    def mac_gen(ms, g, l):
        L = LT(l)
        R = slice(8 * g, 8 * g + 8)
        R2 = slice(B + 8 * g, B + 8 * g + 8)
        G = cfg["G"]
        res = {}
        cnt = 0
        for c in range(3):
            kc = {}
            acc = {m: (None if c == 0 else res[m, 0]) for m in ms}
            for i in range(max(ms) + 1):
                x = XS[i, c, R, L]
                for m in ms:
                    a = m - i
                    if a < 0:
                        continue
                    if a not in kc:
                        kc[a] = KS[a, c, R, L]
                    t = x * kc[a]
                    acc[m] = t if acc[m] is None else (acc[m] - t if c == 2 else acc[m] + t)
                    cnt += 2
                if cnt >= G and not (c == 2 and i == max(ms)):
                    yield cnt, [acc[m] for m in ms if acc[m] is not None]
                    cnt = 0
            for m in ms:
                res[m, c] = acc[m]
        outs = []
        even = g < 8
        for m in ms:
            re, im = res[m, 2], res[m, 1]
            if m > 0:
                if m - 1 in ms:
                    pr, pi = res[m - 1, 2], res[m - 1, 1]
                else:
                    pr, pi = PS[m - 1, R, L], PS[m - 1, R2, L]
                re, im = (re - pi, im + pr) if even else (re + pi, im - pr)
            YS[m, R, L] = re
            YS[m, R2, L] = im
            outs += [re, im]
        m = max(ms)
        if m + 1 < NB:
            PS[m, R, L] = res[m, 2]
            PS[m, R2, L] = res[m, 1]
        for m in ms:
            ymark[m] = ymark.get(m, 0) + 1
        yield cnt + 2 * len(outs), outs

    def push_mac(ms, lo=0, hi=64):
        for i in range(max(ms) + 1):
            assert ("x", i) in ready and ("k", i) in ready, (ms, i)
        for idx in range(lo, hi):
            l, g = idx // 16, idx % 16
            Q["mac"].append(mac_gen(ms, g, l))

    def flush(*names):
        for name in (names or Q):
            q = Q[name]
            if q and cfg.get("verbose"):
                print("  flush", name, len(q))
            while q:
                j = q.pop(0)
                if name == "mac":
                    for _ in j:
                        pass
                else:
                    j[2]()
        st["credit"] = 0.0
        st["maccredit"] = 0.0

    def set_rate(r):
        st["macrate"] = r

    def slot(piece, cap, dt):
        st["credit"] = min(st["credit"] + cap, cfg["maxcredit"])
        st["maccredit"] = min(st["maccredit"] + st["macrate"] * dt, cfg["maxcredit"])
        deps = []
        for name in ("post", "c", "kv"):
            q = Q[name]
            if q and q[0][0] > 0:
                q[0][0] -= 1
                continue
            while q and q[0][0] == 0 and st["credit"] > 0:
                _, cost, thunk = q.pop(0)
                st["credit"] -= cost
                deps += thunk()
        q = Q["mac"]
        while q and st["credit"] > 0 and st["maccredit"] > 0:
            try:
                cost, d = next(q[0])
            except StopIteration:
                q.pop(0)
                continue
            st["credit"] -= cost
            st["maccredit"] -= cost
            deps += d
        if deps:
            d = deps[0]
            for e in deps[1:]:
                d = d + e
            if piece.dtype == u32:
                d = pltpu.bitcast(d, u32)
            w = piece.shape[1]
            piece = jnp.where(st["never"][:, :w], d[:, :w], piece)
        return piece

    def linked_init(init, cap, dt):
        return jnp.concatenate([slot(init[r:r + 8], cap, dt) for r in range(0, init.shape[0], 8)], axis=0)

    def linked_tiles(tiles, cap, dt):
        pieces = [[w[8 * i:8 * i + 8] for i in range(w.shape[0] // 8)] for w in tiles]
        for t0 in range(0, len(tiles), 4):
            for p in range(7, -1, -1):
                for t in range(t0, min(t0 + 4, len(tiles))):
                    if p < len(pieces[t]):
                        pieces[t][p] = slot(pieces[t][p], cap, dt)
        return [jnp.concatenate(ps, axis=0) for ps in pieces]

    def ln(x):
        m = jnp.mean(x, axis=-1, keepdims=True)
        xc = x - m
        var = jnp.mean(xc * xc, axis=-1, keepdims=True)
        return xc * lax.rsqrt(var + EPS)

    def stage_c(b):
        assert not Q["mac"] or ymark.get(b, 0) == 64, (b, ymark.get(b, 0))
        gm = pltpu.bitcast(gu[...], bf16)
        sd = cached("sd", lambda: sdb[...].astype(f32)[None, :])
        r0 = b * B
        ys = []
        for l in range(NL):
            init = linked_init(KV[r0:r0 + B, LT(l)] * sd[:, LT(l)], cfg["capx"] * 4, 4)
            ys.append(jnp.dot(gm, YS[b, :, LT(l)].astype(bf16), preferred_element_type=f32) + init)
        y = jnp.concatenate(ys, axis=1)

        def job(g):
            r0 = b * B + 8 * g
            x = qb[r0:r0 + 8, :].astype(f32)
            h = x + ln(x) * y[8 * g:8 * g + 8]
            HR[r0:r0 + 8, :] = h
            hn = ln(h)
            HN[r0:r0 + 8, :] = hn
            return [hn[:, LT(l)] for l in range(NL)]

        for g in range(16):
            Q["c"].append([cfg["c_delay"] if g == 0 else 0, 76, functools.partial(job, g)])

    def retile_w1():
        w1u[...] = pltpu.bitcast(w1t[...], u32)

    def retile_w2():
        w2u[...] = pltpu.bitcast(w2[...], u32)

    hs = {}

    def stage_f1(b, nb=1, c0=0, c1=NF):
        r0 = b * B
        hn = cached(("hn", b), lambda: HN[r0:r0 + nb * B, :].astype(bf16))
        b1 = cached("b1", lambda: b1b[...].astype(f32)[None, :])
        out = hs.setdefault(b, [])
        dt = 4 * nb
        for c in range(c0, c1):
            lo, hi = c * 128, min((c + 1) * 128, F)
            w = w1u[lo // 2:hi // 2, :]
            init = linked_init(jnp.broadcast_to(b1[:, lo:hi], (nb * B, hi - lo)), cfg["cap1"] * 8, 8)
            t = lax.dot_general(hn, pltpu.bitcast(w, bf16), NT, preferred_element_type=f32) + init
            u = t * (C0 + C1 * (t * t))
            out.append(t + t * jnp.tanh(u))

    def save_h1(b, nb=1):
        H1[b * B:(b + nb) * B, :] = jnp.concatenate(hs.pop(b), axis=1)

    os_ = {}

    def stage_f2(b, nb=1, l0=0, l1=NL):
        r0 = b * B
        if b in hs:
            if isinstance(hs[b], list):
                hs[b] = tuple(jnp.concatenate(hs[b][k0 // 128:(k1 + 127) // 128], axis=1).astype(bf16)
                              for k0, k1 in KG)
        else:
            hs[b] = tuple(H1[r0:r0 + nb * B, k0:k1].astype(bf16) for k0, k1 in KG)
        h = hs[b]
        b2 = cached("b2", lambda: 2.0 * b2b[...].astype(f32)[None, :])
        out = os_.setdefault(b, [])
        dt = 4 * nb
        for l in range(l0, l1):
            o = jnp.broadcast_to(b2[:, LT(l)], (nb * B, 128))
            for (k0, k1), hk in zip(KG, h):
                dt = 8 * (k1 - k0) / 512
                o = jnp.dot(hk, pltpu.bitcast(w2u[k0 // 2:k1 // 2, LT(l)], bf16),
                            preferred_element_type=f32) + linked_init(o, cfg["cap2"] * dt, dt)
            out.append(o)
        if l1 == NL:
            o = jnp.concatenate(os_.pop(b), axis=1)
            hs.pop(b)
            ob[r0:r0 + nb * B, :] = (HR[r0:r0 + nb * B, :] + 0.5 * o).astype(bf16)
            for i in range(nb):
                out_copies[b + i].start()

    ops = dict(tables=tables, kv=push_kv, x=stage_x, k=stage_k, mac=push_mac, flush=flush, c=stage_c,
               f1=stage_f1, f2=stage_f2, rw1=retile_w1, rw2=retile_w2, rate=set_rate, sh1=save_h1)

    for ridx, (waits, region) in enumerate(plan["prog"]):
        for wname in waits:
            for c in groups[wname]:
                c.wait()

        @pl.when(zero != ridx + 1)
        def _(region=region):
            st["never"] = lax.broadcasted_iota(jnp.int32, (8, 128), 0) < zero
            st["cache"] = {}
            for step in region:
                if step[0] == "wait":
                    for c in groups[step[1]]:
                        c.wait()
                else:
                    ops[step[0]](*step[1:])
            left = {k: len(v) for k, v in Q.items() if v}
            if left and cfg.get("verbose"):
                print("region", ridx, "unlinked leftovers:", left)
            flush()
            assert not hs and not os_ and not kvv

    for c in out_copies:
        c.wait()


def default_plan(**over):
    cfg = dict(G=32, cap1=2.0, cap2=2.9, capx=2.5, maxcredit=40, c_delay=24, verbose=False)
    cfg.update(over)
    dma = [("g0", ["small", ("kvs", 0, 2)]), ("q0", [("q", 0, 2)]), ("w1", ["w1"]), ("g1", [("kvsq", 2, 4)]),
           ("w2", ["w2"]), ("g2", [("kvsq", 4, 6)]), ("g3", [("kvsq", 6, 8)]), ("g45", [("kvsq", 8, 12)]),
           ("g67", [("kvsq", 12, 16)])]
    fl = ("flush",)
    kv = lambda p: [("kv", 2 * p), ("kv", 2 * p + 1)]
    K = lambda b: [("k", b)]
    X = lambda b: [("x", b)]
    C = lambda b: [("c", b)]
    M = lambda p, lo=0, hi=64: [("mac", [2 * p, 2 * p + 1], lo, hi)]
    F1 = lambda p, c0, c1: [("f1", 2 * p, 2, c0, c1)]
    F2 = lambda p, l0, l1: [("f2", 2 * p, 2, l0, l1)]
    fm = [("flush", "mac")]
    prog = [
        ([], [("tables",)]),
        (["g0"], kv(0) + K(0) + X(0) + K(1) + X(1) + M(0) + fm + [("wait", "q0")] + C(0) + C(1)),
        (["w1"], [("rw1",)] + F1(0, 0, 8) + [("wait", "g1")] + kv(1) + K(2) + K(3) + F1(0, 8, 9) + X(2) + F1(0, 9, 10)
         + X(3) + M(1) + F1(0, 10, 11) + fm + [("sh1", 0, 2)] + C(2) + C(3)),
        (["w2"], [("rw2",)] + F2(0, 0, 4)),
        (["g2"], kv(2) + K(4) + K(5) + F1(1, 0, 2) + X(4) + F1(1, 2, 4) + X(5) + M(2) + F1(1, 4, 11) + F2(1, 0, 1) + fm
         + C(4) + F2(1, 1, 2) + C(5) + F2(1, 2, 4)),
        (["g3", "g45"], kv(3) + kv(4) + kv(5) + K(6) + K(7) + F1(2, 0, 2) + X(6) + F1(2, 2, 4) + X(7) + M(3)
         + K(8) + K(9) + K(10) + K(11) + F1(2, 4, 11) + X(8) + X(9) + F2(2, 0, 1) + fm + M(4, 0, 16)
         + C(6) + F2(2, 1, 2) + C(7) + X(10) + X(11) + F2(2, 2, 4)),
        (["g67"], M(4, 16, 64) + kv(6) + kv(7) + K(12) + K(13) + K(14) + K(15) + F1(3, 0, 11) + F2(3, 0, 1) + fm
         + M(5, 0, 32) + C(8) + X(12) + X(13) + F2(3, 1, 2) + C(9) + X(14) + X(15) + F2(3, 2, 4)),
        ([], M(5, 32, 64) + F1(4, 0, 9) + fm + M(6, 0, 40) + C(10) + F1(4, 9, 11) + F2(4, 0, 1) + C(11) + F2(4, 1, 4)),
        ([], M(6, 40, 64) + F1(5, 0, 8) + fm + M(7, 0, 36) + C(12) + F1(5, 8, 11) + F2(5, 0, 1) + C(13) + F2(5, 1, 4)),
        ([], M(7, 36, 64) + F1(6, 0, 11) + fm + C(14) + F2(6, 0, 1) + C(15) + F2(6, 1, 4)),
        ([], F1(7, 0, 11) + F2(7, 0, 4)),
    ]
    return dict(dma=dma, prog=prog, cfg=cfg)


def build(plan):
    n_in = sum(4 if it == "small" else (1 if it in ("w1", "w2") else len(it[0])) for _, sp in plan["dma"] for it in sp)

    @jax.jit
    def fn(A_q, A_k, A_v, A_shift_k, A_ssm_k, A_ssm_D, B_x, B_w1, B_b1, B_w2, B_b2):
        ANY = pl.BlockSpec(memory_space=pl.ANY)
        V = pltpu.VMEM
        scratch = [
            V((S, D), bf16), V((S, D), bf16), V((S, D), bf16), V((D, S), bf16),
            V((F, D), bf16), V((F, D), bf16),
            V((4, D), bf16), V((D,), bf16), V((F,), bf16), V((D,), bf16),
            V((NL, S + 8, 128), f32), V((S, D), bf16),
            V((F // 2, D), u32), V((F // 2, D), u32),
            V((B, B), u32), V((B // 2, 2 * B), u32),
            V((NB, 3, B, D), f32), V((NB, 3, B, D), f32), V((NB, 2 * B, D), f32),
            V((S, D), f32), V((S, D), f32), V((NB, 2 * B, D), f32), V((S, D), f32),
            V((4 * B, F), f32),
            pltpu.SemaphoreType.DMA((n_in,)), pltpu.SemaphoreType.DMA((NB,)),
            pltpu.SemaphoreType.REGULAR((1,)),
        ]
        out = pl.pallas_call(
            functools.partial(_kernel, plan=plan),
            in_specs=[ANY] * 10,
            out_specs=ANY,
            out_shape=jax.ShapeDtypeStruct((S, D), bf16),
            scratch_shapes=scratch,
            compiler_params=pltpu.CompilerParams(vmem_limit_bytes=120 * 1024 * 1024),
        )(A_q.reshape(S, D), A_k.reshape(S, D), A_v.reshape(S, D), A_shift_k.T, A_ssm_k, A_ssm_D,
          B_w1.T, B_b1, B_w2, B_b2)
        return out.reshape(1, S, D)

    return fn


_PLAN = default_plan()
_FN = build(_PLAN)


def pallas_sequential_preLN__ssm_conv_h3__dense_activation_gelu__prompt_kernel(A_q, A_k, A_v, A_shift_k, A_ssm_k, A_ssm_D, B_x, B_w1, B_b1, B_w2, B_b2):
    return _FN(A_q, A_k, A_v, A_shift_k, A_ssm_k, A_ssm_D, B_x, B_w1, B_b1, B_w2, B_b2)
```

```python
import contextlib
import functools
import math

import jax
import jax.numpy as jnp
from jax import lax
import jax.experimental.pallas as pl
import jax.experimental.pallas.tpu as pltpu

S, D, F = 2048, 512, 1376
B = 128
NB = S // B
NL = D // 128
NF = (F + 127) // 128
EPS = 1e-5
f32, bf16, u32 = jnp.float32, jnp.bfloat16, jnp.uint32
NT = (((1,), (1,)), ((), ()))
C0 = math.sqrt(2.0 / math.pi)
C1 = C0 * 0.044715
KG = ((0, 512), (512, 1024), (1024, F))
BETA = C1 ** (1.0 / 3.0)
KAPPA = C0 / BETA
GAMMA = 0.5 / BETA


def _kernel(q_hbm, k_hbm, v_hbm, sk_hbm, ssm_hbm, sd_hbm, w1t_hbm, b1_hbm, w2_hbm, b2_hbm,
            o_hbm,
            qb, kb, vb, ssm, w1t, w2, skb, sdb, b1b, b2b, kf, ob,
            w1u, w2u, fu, gu, XS, KS, PS, HR, YS, HN, H1, YT,
            zs, isem, osem, *, plan):
    cfg = dict(plan["cfg"])
    pid = pl.program_id(0)

    sem_id = [0]

    def cp(src, dst):
        return pltpu.make_async_copy(src, dst, isem.at[sem_id[0]])

    def blk_copies(b0, b1):
        r = pl.ds(b0 * B, (b1 - b0) * B)
        return [cp(k_hbm.at[r], kb.at[r]), cp(v_hbm.at[r], vb.at[r]),
                cp(ssm_hbm.at[:, r], ssm.at[:, r]), cp(q_hbm.at[r], qb.at[r])]

    groups = {}
    for name, spec in plan["dma"]:
        cs = []
        for item in spec:
            if item == "sk":
                cs += [cp(sk_hbm, skb), cp(sd_hbm, sdb)]
            elif item == "small":
                cs += [cp(b1_hbm, b1b), cp(b2_hbm, b2b)]
            elif item[0] in ("w1", "w2"):
                src, dst = (w1t_hbm, w1t) if item[0] == "w1" else (w2_hbm, w2)
                r = pl.ds(item[1] * 128, min(item[2] * 128, F) - item[1] * 128)
                cs += [cp(src.at[r], dst.at[r])]
            else:
                r = pl.ds(item[1] * B, (item[2] - item[1]) * B)
                for ch in item[0]:
                    if ch == "s":
                        cs.append(cp(ssm_hbm.at[:, r], ssm.at[:, r]))
                    else:
                        src, dst = dict(k=(k_hbm, kb), v=(v_hbm, vb), q=(q_hbm, qb))[ch]
                        cs.append(cp(src.at[r], dst.at[r]))
        groups[name] = cs
        sem_id[0] += 1

    def start_dmas():
        for cs in groups.values():
            for c in cs:
                c.start()

    def out_copy(b, nb):
        r = pl.ds(b * B, nb * B)
        return pltpu.make_async_copy(ob.at[r], o_hbm.at[r], osem.at[0])

    Q = dict(post=[], c=[], kv=[], mac=[])
    st = dict(credit=0.0, never=None, cache={}, macrate=1e9, maccredit=0.0)

    def cached(key, fn):
        if key not in st["cache"]:
            st["cache"][key] = fn()
        return st["cache"][key]

    def LT(l):
        return slice(l * 128, (l + 1) * 128)

    def tables():
        start_dmas()
        zs[0] = 0

        def cosn(n, scale):
            n = jnp.abs((n & (4 * B - 1)) - 2 * B)
            x = (n - B).astype(f32) * (2.0 * math.pi / (4 * B))
            x2 = x * x
            p = -1.0 / 39916800.0
            for cf in (1.0 / 362880.0, -1.0 / 5040.0, 1.0 / 120.0, -1.0 / 6.0, 1.0):
                p = p * x2 + cf
            return p * (x * scale)

        r = lax.broadcasted_iota(jnp.int32, (2 * B, B), 0)
        j = lax.broadcasted_iota(jnp.int32, (2 * B, B), 1)
        slot_ = ((r >> 5) << 4) + (r & 15)
        odd = jnp.where(slot_ < B // 2, 4 * slot_ + 1, 4 * B - 1 - 4 * slot_)
        fu[...] = pltpu.bitcast(cosn(odd * j + ((r & 16) << 3), 1.0).astype(bf16), u32)
        r = lax.broadcasted_iota(jnp.int32, (B, B), 0)
        c = lax.broadcasted_iota(jnp.int32, (B, B), 1)
        j = 2 * (r & (B // 2 - 1)) + (r >> 6)
        gu[...] = pltpu.bitcast(
            cosn((4 * (c & (B // 2 - 1)) + 1) * j + ((c & (B // 2)) << 1), 1.0 / B).astype(bf16), u32)
        for l in range(NL):
            kf[l, 0:8, :] = jnp.zeros((8, 128), f32)

    kvv = {}
    ymark = {}

    def ku_job(b, g):
        r0 = b * B + 16 * g
        kall = kb[r0:r0 + 16, :].astype(f32)
        for l in range(NL):
            kf[l, 8 + r0:24 + r0, :] = kall[:, LT(l)]
        return [kall[8:16, LT(NL - 1)]]

    def kv_job(b, g):
        r0 = b * B + 8 * g
        sk = cached("sk", lambda: skb[...].astype(f32))
        vall = vb[r0:r0 + 8, :].astype(f32)
        outs = []
        for l in range(NL):
            acc = kf[l, 8 + r0:16 + r0, :] * sk[0:1, LT(l)]
            for t in range(1, 4):
                acc = acc + kf[l, 8 + r0 - t:16 + r0 - t, :] * sk[t:t + 1, LT(l)]
            outs.append(acc * vall[:, LT(l)])
        kv = jnp.concatenate(outs, axis=1)
        kvv.setdefault(b, []).append(kv)
        return outs

    def push_kv(*bs):
        for b in bs:
            for g in range(8):
                Q["kv"].append([0, 12, functools.partial(ku_job, b, g)])
        for b in bs:
            for g in range(16):
                Q["kv"].append([0, 40, functools.partial(kv_job, b, g)])

    ready = set()

    def split_ri(h, g):
        r0 = (g // 2) * 32 + (g % 2) * 8
        return h[r0:r0 + 8], h[r0 + 16:r0 + 24]

    def stage_x(b):
        while Q["kv"] and len(kvv.get(b, [])) < 16:
            Q["kv"].pop(0)[2]()
        kv = jnp.concatenate(kvv.pop(b), axis=0)
        fm = pltpu.bitcast(fu[...], bf16)
        xh = jnp.dot(fm, kv.astype(bf16), preferred_element_type=f32)
        for g in range(16):
            a, bb = split_ri(xh, g)
            R = slice(8 * g, 8 * g + 8)
            XS[b, 1, R, :] = a
            XS[b, 2, R, :] = bb
            a = jnp.concatenate([slot(a[:, LT(l)], cfg["capx"] * 4, 4) for l in range(NL)], axis=1)
            XS[b, 0, R, :] = a + bb
        ready.add(("x", b))

    def stage_k(a):
        fm = pltpu.bitcast(fu[...], bf16)
        kh = lax.dot_general(fm, ssm[:, a * B:(a + 1) * B], NT, preferred_element_type=f32)
        for g in range(16):
            c, d = split_ri(kh, g)
            if a == 0:
                c = c + cached("sd", lambda: sdb[...].astype(f32)[None, :])
            R = slice(8 * g, 8 * g + 8)
            KS[a, 0, R, :] = c
            c = jnp.concatenate([slot(c[:, LT(l)], cfg["capx"] * 4, 4) for l in range(NL)], axis=1)
            KS[a, 1, R, :] = d - c
            KS[a, 2, R, :] = c + d
        ready.add(("k", a))

    def mac_gen(terms, first, last, g, l):
        L = LT(l)
        R = slice(8 * g, 8 * g + 8)
        R2 = slice(B + 8 * g, B + 8 * g + 8)
        G = cfg["G"]
        ms = sorted(terms)
        iis = sorted(set(i for m in ms for i in terms[m]))
        res = {}
        cnt = 0
        for c in range(3):
            kc = {}
            acc = {}
            for m in ms:
                if c == 0:
                    acc[m] = None
                elif first[m]:
                    acc[m] = res[m, 0]
                else:
                    acc[m] = res[m, 0] + PS[m, R2 if c == 1 else R, L]
                    cnt += 1
            for i in iis:
                x = XS[i, c, R, L]
                for m in ms:
                    if i not in terms[m]:
                        continue
                    a = m - i
                    if a not in kc:
                        kc[a] = KS[a, c, R, L]
                    t = x * kc[a]
                    acc[m] = t if acc[m] is None else (acc[m] - t if c == 2 else acc[m] + t)
                    cnt += 2
                if cnt >= G and not (c == 2 and i == iis[-1]):
                    yield cnt, [acc[m] for m in ms if acc[m] is not None]
                    cnt = 0
            for m in ms:
                res[m, c] = acc[m]
        outs = []
        even = g < 8
        for m in ms:
            re, im = res[m, 2], res[m, 1]
            if not (last[m] and (m + 1 == NB or (m + 1 in ms and last[m + 1]))):
                PS[m, R, L] = re
                PS[m, R2, L] = im
            if last[m]:
                if m > 0:
                    if m - 1 in ms:
                        assert last[m - 1]
                        pr, pi = res[m - 1, 2], res[m - 1, 1]
                    else:
                        pr, pi = PS[m - 1, R, L], PS[m - 1, R2, L]
                    re, im = (re - pi, im + pr) if even else (re + pi, im - pr)
                YS[m, R, L] = re
                YS[m, R2, L] = im
                ymark[m] = ymark.get(m, 0) + 1
            outs += [re, im]
        yield cnt + 2 * len(outs), outs

    prio = {}
    tdone = {}

    def push_mac(ms, lim=NB, lo=0, hi=64):
        for idx in range(lo, hi):
            l, g = idx // 16, idx % 16
            terms, first, last = {}, {}, {}
            for m in ms:
                done = tdone.setdefault((m, idx), set())
                t = [i for i in range(m + 1) if i <= lim and m - i <= lim and i not in done]
                if not t:
                    continue
                for i in t:
                    assert ("x", i) in ready and ("k", m - i) in ready, (m, i)
                terms[m], first[m] = t, not done
                done.update(t)
                last[m] = len(done) == m + 1
                if last[m] and m > 0 and m - 1 not in ms:
                    assert len(tdone[m - 1, idx]) == m
            if terms:
                gen = mac_gen(terms, first, last, g, l)
                prio[id(gen)] = min(ms)
                Q["mac"].append(gen)
        q = Q["mac"]
        head = q[:1] if q and st.get("open") is q[0] else []
        q[:] = head + sorted(q[len(head):], key=lambda gn: prio[id(gn)])

    def flush(*names):
        for name in (names or Q):
            q = Q[name]
            if q and cfg.get("verbose"):
                print("  flush", name, len(q))
            while q:
                j = q.pop(0)
                if name == "mac":
                    for _ in j:
                        pass
                else:
                    j[2]()
        st["credit"] = 0.0
        st["maccredit"] = 0.0

    def set_rate(r):
        st["macrate"] = r

    def slot(piece, cap, dt):
        if st["never"] is None:
            return piece
        st["credit"] = min(st["credit"] + cap, cfg["maxcredit"])
        st["maccredit"] = min(st["maccredit"] + st["macrate"] * dt, cfg["maxcredit"])
        deps = []
        for name in ("post", "c", "kv"):
            q = Q[name]
            if name == "c" and st.get("hold"):
                continue
            if q and q[0][0] > 0:
                q[0][0] -= 1
                continue
            while q and q[0][0] == 0 and st["credit"] > 0:
                _, cost, thunk = q.pop(0)[:3]
                st["credit"] -= cost
                deps += thunk()
        q = Q["mac"]
        while q and st["credit"] > 0 and st["maccredit"] > 0:
            try:
                st["open"] = q[0]
                cost, d = next(q[0])
            except StopIteration:
                q.pop(0)
                continue
            st["credit"] -= cost
            st["maccredit"] -= cost
            deps += d
        if deps:
            d = deps[0]
            for e in deps[1:]:
                d = d + e
            if piece.dtype == u32:
                d = pltpu.bitcast(d, u32)
            w = piece.shape[1]
            piece = jnp.where(st["never"][:, :w], d[:, :w], piece)
        return piece

    def linked_init(init, cap, dt):
        return jnp.concatenate([slot(init[r:r + 8], cap, dt) for r in range(0, init.shape[0], 8)], axis=0)

    def linked_tiles(tiles, cap, dt):
        pieces = [[w[8 * i:8 * i + 8] for i in range(w.shape[0] // 8)] for w in tiles]
        for t0 in range(0, len(tiles), 4):
            for p in range(7, -1, -1):
                for t in range(t0, min(t0 + 4, len(tiles))):
                    if p < len(pieces[t]):
                        pieces[t][p] = slot(pieces[t][p], cap, dt)
        return [jnp.concatenate(ps, axis=0) for ps in pieces]

    def ln(x, scale=1.0):
        m = jnp.mean(x, axis=-1, keepdims=True)
        xc = x - m
        ss = jnp.sum(xc * xc, axis=-1, keepdims=True)
        if cfg.get("explog", True):
            r = jnp.exp(math.log(scale * math.sqrt(D)) - 0.5 * jnp.log(ss + D * EPS))
        else:
            r = lax.rsqrt(ss * (1.0 / (D * scale * scale)) + EPS / (scale * scale))
        return xc * r

    def stage_c(b):
        if ymark.get(b, 0) < 64 and cfg.get("verbose"):
            print("  stage_c", b, "forces", 64 - ymark.get(b, 0), "mac chunks")
        while ymark.get(b, 0) < 64:
            for _ in Q["mac"].pop(0):
                pass
        gm = pltpu.bitcast(gu[...], bf16)
        H = B // 2
        for l in range(NL):
            re0, re1 = YS[b, 0:H, LT(l)], YS[b, H:B, LT(l)]
            im0, im1 = YS[b, B:B + H, LT(l)], YS[b, B + H:2 * B, LT(l)]
            u = jnp.concatenate([re0 + re1, im0 - im1], axis=0).astype(bf16)
            v = jnp.concatenate([re0 - re1, im0 + im1], axis=0).astype(bf16)
            YT[l, pl.ds(b * B, H, stride=2), :] = jnp.dot(gm[:H], u, preferred_element_type=f32)
            YT[l, pl.ds(b * B + 1, H, stride=2), :] = jnp.dot(gm[H:], v, preferred_element_type=f32)

        def job(g):
            r0 = b * B + 8 * g
            x = qb[r0:r0 + 8, :].astype(f32)
            h = x + ln(x) * jnp.concatenate([YT[l, r0:r0 + 8, :] for l in range(NL)], axis=1)
            HR[r0:r0 + 8, :] = h
            hn = ln(h, BETA)
            HN[r0:r0 + 8, :] = hn
            return [hn[:, LT(l)] for l in range(cfg.get("clink", NL))]

        for g in range(16):
            Q["c"].append([cfg["c_delay"] if g == 0 else 0, 68, functools.partial(job, g), b])

    def retile_w1(c0=0, c1=NF):
        lo, hi = c0 * 128, min(c1 * 128, F)
        w1u[lo // 2:hi // 2, :] = pltpu.bitcast(w1t[lo:hi, :], u32)

    def retile_w2():
        w2u[...] = pltpu.bitcast(w2[...], u32)

    hs = {}

    def stage_f1(b, nb=1, c0=0, c1=NF, save=False):
        r0 = b * B
        while any(j[3] in range(b, b + nb) for j in Q["c"]):
            if cfg.get("verbose"):
                print("  f1", b, "forces c job")
            Q["c"].pop(0)[2]()
        hn = cached(("hn", b), lambda: HN[r0:r0 + nb * B, :].astype(bf16))
        b1 = cached("b1", lambda: BETA * b1b[...].astype(f32)[None, :])
        out = [] if save else hs.setdefault(b, [])
        for c in range(c0, c1):
            lo, hi = c * 128, min((c + 1) * 128, F)
            w = w1u[lo // 2:hi // 2, :]
            init = linked_init(jnp.broadcast_to(b1[:, lo:hi], (nb * B, hi - lo)), cfg["cap1"] * 8, 8)
            t = lax.dot_general(hn, pltpu.bitcast(w, bf16), NT, preferred_element_type=f32) + init
            u = t * (KAPPA + t * t)
            out.append(t + t * jnp.tanh(u))
            if save:
                H1[r0:r0 + nb * B, lo:hi] = out[-1]

    def save_h1(b, nb=1):
        H1[b * B:(b + nb) * B, :] = jnp.concatenate(hs.pop(b), axis=1)

    os_ = {}

    def stage_f2(b, nb=1, l0=0, l1=NL):
        r0 = b * B
        if b in hs:
            if isinstance(hs[b], list):
                hs[b] = tuple(jnp.concatenate(hs[b][k0 // 128:(k1 + 127) // 128], axis=1).astype(bf16)
                              for k0, k1 in KG)
        else:
            hs[b] = tuple(H1[r0:r0 + nb * B, k0:k1].astype(bf16) for k0, k1 in KG)
        h = hs[b]
        b2 = cached("b2", lambda: (1.0 / GAMMA) * b2b[...].astype(f32)[None, :])
        out = os_.setdefault(b, [])
        dt = 4 * nb
        for l in range(l0, l1):
            o = jnp.broadcast_to(b2[:, LT(l)], (nb * B, 128))
            for (k0, k1), hk in zip(KG, h):
                dt = 8 * (k1 - k0) / 512
                o = jnp.dot(hk, pltpu.bitcast(w2u[k0 // 2:k1 // 2, LT(l)], bf16),
                            preferred_element_type=f32) + linked_init(o, cfg["cap2"] * dt, dt)
            out.append(o)
        if l1 == NL:
            o = jnp.concatenate(os_.pop(b), axis=1)
            hs.pop(b)
            ob[r0:r0 + nb * B, :] = (HR[r0:r0 + nb * B, :] + GAMMA * o).astype(bf16)
            out_copy(b, nb).start()

    ops = dict(hold=lambda v: st.update(hold=v), set=lambda k, v: cfg.update({k: v}), tables=tables, kv=push_kv, x=stage_x, k=stage_k, mac=push_mac, flush=flush, c=stage_c,
               f1=stage_f1, f2=stage_f2, rw1=retile_w1, rw2=retile_w2, rate=set_rate, sh1=save_h1)

    nreg = len(plan["prog"])
    for ridx, region in enumerate(plan["prog"]):
        def body(region=region, ridx=ridx):
            if ridx > 0:
                st["never"] = lax.broadcasted_iota(jnp.int32, (8, 128), 0) < zs[0]
            st["cache"] = {}
            for step in region:
                if step[0] == "wait":
                    with jax.named_scope(f"wait_{step[1]}") if cfg.get("scopes") else contextlib.nullcontext():
                        for c in groups[step[1]]:
                            c.wait()
                else:
                    ops[step[0]](*step[1:])
            left = {k: len(v) for k, v in Q.items() if v}
            if left and cfg.get("verbose"):
                print("region", ridx, "unlinked leftovers:", left)
            if Q["mac"] and st.get("open") is Q["mac"][0]:
                for _ in Q["mac"].pop(0):
                    pass
            flush("post", "c", "kv")
            if ridx == nreg - 1:
                assert not Q["mac"]
            assert not hs and not os_ and not kvv
            if ridx == nreg - 1:
                out_copy(0, NB).wait()

        with jax.named_scope(f"region_{ridx}") if cfg.get("scopes") else contextlib.nullcontext():
            pl.when(pid == ridx)(body)


def default_plan(**over):
    cfg = dict(G=32, cap1=1.8, cap2=2.2, capx=2.0, maxcredit=40, c_delay=24, scap1=2.2, scapx=2.5, verbose=False)
    cfg.update(over)
    n1 = cfg.get("n1", 5)
    dma = [("a0", ["sk", ("kvs", 0, 1)]), ("a1", [("kvs", 1, 2)]), ("q0", [("q", 0, 2), "small"]),
           ("g1", [("kvs", 2, 4)]), ("w1a", [("w1", 0, n1)]), ("w1b", [("q", 2, 4), ("w1", n1, 11)]),
           ("g2", [("kvsq", 4, 6)]), ("w2", [("w2", 0, 11)]), ("g3", [("kvsq", 6, 8)]),
           ("g4", [("kvs", 8, 16)]), ("q4", [("q", 8, 16)])]
    W = lambda n: [("wait", n)]
    kv = lambda *ps: [("kv", *[b for p in ps for b in (2 * p, 2 * p + 1)])]
    K = lambda b: [("k", b)]
    X = lambda b: [("x", b)]
    C = lambda b: [("c", b)]
    M = lambda p, lim=NB, lo=0, hi=64: [("mac", [2 * p, 2 * p + 1], lim, lo, hi)]
    F1 = lambda p, c0, c1, save=False: [("f1", 2 * p, 2, c0, c1, save)]
    S1 = lambda p, c0, c1: F1(p, c0, c1, True)
    F2 = lambda p, l0, l1: [("f2", 2 * p, 2, l0, l1)]
    M1 = lambda m: [("mac", [m])]

    def FC(p):
        v = cfg.get("cpos", 3)
        b = 2 * p + 2
        if v == 0:
            return F1(p, 0, 8) + C(b) + F1(p, 8, 11) + C(b + 1) + F2(p, 0, 4)
        if v == 1:
            return F1(p, 0, 11) + F2(p, 0, 1) + C(b) + F2(p, 1, 2) + C(b + 1) + F2(p, 2, 4)
        if v == 2:
            return F1(p, 0, 11) + F2(p, 0, 2) + C(b) + C(b + 1) + F2(p, 2, 4)
        if v == 3:
            return F1(p, 0, 11) + F2(p, 0, 1) + C(b) + C(b + 1) + F2(p, 1, 4)
    prog = [
        [("tables",)] + W("a0") + [("kv", 0)] + K(0) + X(0) + M1(0) + [("flush",)],
        W("a1") + [("hold", True), ("set", "cap1", cfg["scap1"]), ("set", "capx", cfg["scapx"]), ("kv", 1)]
        + K(1) + X(1) + M1(1) + C(0) + C(1)
        + W("q0") + W("g1") + [("hold", False)] + K(2) + K(3) + kv(1) + X(2) + X(3),
        W("w1a") + [("rw1", 0, n1), ("hold", True)] + M(1) + S1(0, 0, n1 - 1) + C(2) + S1(0, n1 - 1, n1) + C(3)
        + W("w1b") + [("rw1", n1, 11), ("hold", False)] + S1(0, n1, 11),
        W("g2") + [("set", "cap1", cfg["cap1"]), ("set", "capx", cfg["capx"])] + kv(2) + M(2, 3) + S1(1, 0, 2) + K(4) + S1(1, 2, 4) + K(5) + S1(1, 4, 6) + X(4) + S1(1, 6, 8) + X(5)
        + S1(1, 8, 11),
        W("w2") + W("g3") + [("rw2",)] + M(2) + M(3, 5) + M(4, 5) + F2(0, 0, 2) + C(4) + F2(0, 2, 3) + C(5) + F2(0, 3, 4)
        + kv(3) + K(6) + F2(1, 0, 1) + K(7) + F2(1, 1, 2) + X(6) + F2(1, 2, 3) + X(7) + F2(1, 3, 4),
        W("g4") + M(3) + M(4, 7) + M(5, 7) + M(6, 7) + F1(2, 0, 2) + K(8) + F1(2, 2, 4) + K(9) + F1(2, 4, 5) + K(10)
        + F1(2, 5, 6) + K(11) + F1(2, 6, 7) + C(6) + F1(2, 7, 8) + K(12) + F1(2, 8, 9) + K(13) + F1(2, 9, 10) + C(7)
        + kv(4, 5, 6, 7) + F1(2, 10, 11) + K(14) + F2(2, 0, 1) + X(8) + K(15) + X(9) + F2(2, 1, 2)
        + X(10) + X(11) + F2(2, 2, 3) + X(12) + X(13) + F2(2, 3, 4) + X(14) + X(15),
        W("q4") + M(4) + M(5) + M(6) + M(7) + FC(3) + FC(4) + FC(5) + FC(6)
        + [("f1", 14, 1, 0, 11, False), ("f1", 15, 1, 0, 11, False), ("f2", 14, 1, 0, 4), ("f2", 15, 1, 0, 4)],
    ]
    return dict(dma=dma, prog=prog, cfg=cfg)


def build(plan):
    n_in = len(plan["dma"])

    @jax.jit
    def fn(A_q, A_k, A_v, A_shift_k, A_ssm_k, A_ssm_D, B_x, B_w1, B_b1, B_w2, B_b2):
        ANY = pl.BlockSpec(memory_space=pl.ANY)
        V = pltpu.VMEM
        scratch = [
            V((S, D), bf16), V((S, D), bf16), V((S, D), bf16), V((D, S), bf16),
            V((F, D), bf16), V((F, D), bf16),
            V((4, D), bf16), V((D,), bf16), V((F,), bf16), V((D,), bf16),
            V((NL, S + 8, 128), f32), V((S, D), bf16),
            V((F // 2, D), u32), V((F // 2, D), u32),
            V((B, B), u32), V((B // 2, B), u32),
            V((NB, 3, B, D), f32), V((NB, 3, B, D), f32), V((NB, 2 * B, D), f32),
            V((S, D), f32), V((NB, 2 * B, D), f32), V((S, D), f32),
            V((S, F), f32), V((NL, S, 128), f32),
            pltpu.SMEM((1,), jnp.int32),
            pltpu.SemaphoreType.DMA((n_in,)), pltpu.SemaphoreType.DMA((1,)),
        ]
        out = pl.pallas_call(
            functools.partial(_kernel, plan=plan),
            grid=(len(plan["prog"]),),
            in_specs=[ANY] * 10,
            out_specs=ANY,
            out_shape=jax.ShapeDtypeStruct((S, D), bf16),
            scratch_shapes=scratch,
            compiler_params=pltpu.CompilerParams(
                dimension_semantics=("arbitrary",), vmem_limit_bytes=120 * 1024 * 1024,
                disable_semaphore_checks=True, disable_bounds_checks=True),
        )(A_q.reshape(S, D), A_k.reshape(S, D), A_v.reshape(S, D), A_shift_k.T, A_ssm_k, A_ssm_D,
          B_w1.T, B_b1, B_w2, B_b2)
        return out.reshape(1, S, D)

    return fn


_PLAN = default_plan()
_FN = build(_PLAN)


def pallas_sequential_preLN__ssm_conv_h3__dense_activation_gelu__prompt_kernel(A_q, A_k, A_v, A_shift_k, A_ssm_k, A_ssm_D, B_x, B_w1, B_b1, B_w2, B_b2):
    return _FN(A_q, A_k, A_v, A_shift_k, A_ssm_k, A_ssm_D, B_x, B_w1, B_b1, B_w2, B_b2)
```

```python
import functools
import math

import jax
import jax.numpy as jnp
from jax import lax
import jax.experimental.pallas as pl
import jax.experimental.pallas.tpu as pltpu

S, D, F = 2048, 512, 1376
B = 128
NB = S // B
SB = 256
NP = S // SB
NL = D // 128
NF = (F + 127) // 128
EPS = 1e-5
f32, bf16, u32 = jnp.float32, jnp.bfloat16, jnp.uint32
NT = (((1,), (1,)), ((), ()))
C0 = math.sqrt(2.0 / math.pi)
C1 = C0 * 0.044715
KG = ((0, 512), (512, 1024), (1024, F))
BETA = C1 ** (1.0 / 3.0)
KAPPA = C0 / BETA
GAMMA = 0.5 / BETA


def _kernel(q_hbm, k_hbm, v_hbm, sk_hbm, ssm_hbm, sd_hbm, w1t_hbm, b1_hbm, w2_hbm, b2_hbm,
            o_hbm,
            qb, kb, vb, ssm, w1t, w2, skb, sdb, b1b, b2b, kf, ob,
            w1u, w2u, fe, fo, gu, XS, KS, PS, YS, HR, HN, H1, YT, KT, XN,
            zs, isem, osem, *, plan):
    cfg = dict(plan["cfg"])
    pid = pl.program_id(0)

    groups = {}
    for gi, (name, spec) in enumerate(plan["dma"]):
        cp = lambda src, dst: pltpu.make_async_copy(src, dst, isem.at[gi])
        cs = []
        for item in spec:
            if item == "sk":
                cs += [cp(sk_hbm, skb), cp(sd_hbm, sdb)]
            elif item == "small":
                cs += [cp(b1_hbm, b1b), cp(b2_hbm, b2b)]
            elif item[0] in ("w1", "w2"):
                src, dst = (w1t_hbm, w1t) if item[0] == "w1" else (w2_hbm, w2)
                r = pl.ds(item[1] * 128, min(item[2] * 128, F) - item[1] * 128)
                cs += [cp(src.at[r], dst.at[r])]
            else:
                r = pl.ds(item[1] * SB, (item[2] - item[1]) * SB)
                for ch in item[0]:
                    if ch == "s":
                        cs.append(cp(ssm_hbm.at[:, r], ssm.at[:, r]))
                    else:
                        src, dst = dict(k=(k_hbm, kb), v=(v_hbm, vb), q=(q_hbm, qb))[ch]
                        cs.append(cp(src.at[r], dst.at[r]))
        groups[name] = cs

    def out_copy(b, nb):
        r = pl.ds(b * B, nb * B)
        return pltpu.make_async_copy(ob.at[r], o_hbm.at[r], osem.at[0])

    Q = dict(c=[], kt=[], kv=[], lq=[], mac=[])
    st = dict(credit=0.0, never=None, cache={}, hold=False, cur=None)

    def cached(key, fn):
        if key not in st["cache"]:
            st["cache"][key] = fn()
        return st["cache"][key]

    def LT(l):
        return slice(l * 128, (l + 1) * 128)

    def tables():
        for cs in groups.values():
            for c in cs:
                c.start()
        zs[0] = 0

        def cosn(n, scale):
            n = jnp.abs((n & 1023) - 512)
            x = (n - 256).astype(f32) * (2.0 * math.pi / 1024)
            x2 = x * x
            p = -1.0 / 39916800.0
            for cf in (1.0 / 362880.0, -1.0 / 5040.0, 1.0 / 120.0, -1.0 / 6.0, 1.0):
                p = p * x2 + cf
            return p * (x * scale)

        r = lax.broadcasted_iota(jnp.int32, (256, 128), 0)
        c = lax.broadcasted_iota(jnp.int32, (256, 128), 1)
        slot_ = ((r >> 5) << 4) + (r & 15)
        odd = jnp.where(slot_ < 64, 4 * slot_ + 1, 511 - 4 * slot_)
        ne = odd * (2 * c) + ((r & 16) << 4)
        fe[...] = pltpu.bitcast(cosn(ne, 1.0).astype(bf16), u32)
        fo[...] = pltpu.bitcast(cosn(ne + odd, 1.0).astype(bf16), u32)
        j = 4 * (r & 63) + (r >> 6)
        gu[...] = pltpu.bitcast(cosn((4 * (c & 63) + 1) * j + ((c & 64) << 2), 1.0 / 256).astype(bf16), u32)
        for l in range(NL):
            kf[l, 0:8, :] = jnp.zeros((8, 128), f32)

    def slot(piece, cap):
        if st["never"] is None:
            return piece
        st["credit"] = min(st["credit"] + cap * cfg["mul"], cfg["maxcredit"])
        deps = []
        for name in ("c", "kt", "kv", "lq"):
            q = Q[name]
            if name == "c" and st["hold"]:
                continue
            if q and q[0][0] > 0:
                q[0][0] -= 1
                continue
            while q and q[0][0] == 0 and st["credit"] > 0:
                j = q.pop(0)
                st["credit"] -= j[1]
                deps += j[2]()
        q = Q["mac"]
        while q and st["credit"] > 0:
            st["cur"] = q[0]
            nxt = next(q[0][1], None)
            if nxt is None:
                q.pop(0)
                continue
            st["credit"] -= nxt[0]
            deps += nxt[1]
        if deps:
            d = deps[0]
            for e in deps[1:]:
                d = d + e
            w = piece.shape[1]
            piece = jnp.where(st["never"][:, :w], d[:, :w], piece)
        return piece

    def linked_init(init, cap):
        return jnp.concatenate([slot(init[r:r + 8], cap) for r in range(0, init.shape[0], 8)], axis=0)

    def force(name, tag):
        while any(j[3] == tag for j in Q[name]):
            Q[name].pop(0)[2]()

    def finish_mac():
        for _ in Q["mac"].pop(0)[1]:
            pass

    kvv = {}

    def ku_job(r0):
        kall = kb[r0:r0 + 16, :].astype(f32)
        for l in range(NL):
            kf[l, 8 + r0:24 + r0, :] = kall[:, LT(l)]
        return [kall[8:16, LT(NL - 1)]]

    def kv_job(p, g, ls):
        r0 = p * SB + 16 * g
        sk = cached("sk", lambda: skb[...].astype(f32))
        outs = []
        for l in ls:
            vw = pltpu.bitcast(vb[r0:r0 + 16, LT(l)], u32)
            ve = pltpu.bitcast(vw << 16, f32)
            vo = pltpu.bitcast(vw & jnp.uint32(0xFFFF0000), f32)
            a = {o: kf[l, pl.ds(8 + r0 + o, 8, stride=2), :] for o in range(-3, 2)}
            w = [sk[t:t + 1, LT(l)] for t in range(4)]
            e = (a[0] * w[0] + a[-1] * w[1] + a[-2] * w[2] + a[-3] * w[3]) * ve
            o = (a[1] * w[0] + a[0] * w[1] + a[-1] * w[2] + a[-2] * w[3]) * vo
            kvv.setdefault((p, l), []).append((e, o))
            outs += [e, o]
        return outs

    def push_kv(*ps):
        for p in ps:
            for g in range(16):
                Q["kv"].append([0, 20, functools.partial(ku_job, p * SB + 16 * g), p])
        for p in ps:
            for g in range(16):
                for ls in ((0, 1), (2, 3)):
                    Q["kv"].append([0, 56, functools.partial(kv_job, p, g, ls), p])

    def kt_job(t0, l):
        t = jnp.transpose(ssm[LT(l), t0:t0 + 128].astype(f32))
        KT[l, t0:t0 + 128, :] = t
        return [t[120:128]]

    def push_kt(*ps):
        for p in ps:
            for l in range(NL):
                for h in range(2):
                    Q["kt"].append([0, 60, functools.partial(kt_job, p * SB + h * 128, l), p])

    ready = set()

    def fwd(p, ls, src, dst, is_k):
        fem, fom = pltpu.bitcast(fe[...], bf16), pltpu.bitcast(fo[...], bf16)
        res = {}
        for l in ls:
            ze, zo = src(l)
            res[l] = (jnp.dot(fem, ze.astype(bf16), preferred_element_type=f32),
                      jnp.dot(fom, zo.astype(bf16), preferred_element_type=f32))
        for g in range(16):
            r0 = (g // 2) * 32 + (g % 2) * 8
            for l in ls:
                e, o = res[l]
                er, ei, orr, oi = e[r0:r0 + 8], e[r0 + 16:r0 + 24], o[r0:r0 + 8], o[r0 + 16:r0 + 24]
                if is_k and p == 0:
                    er = er + cached("sd", lambda: sdb[...].astype(f32)[None, :])[:, LT(l)]
                er = slot(er, cfg["capx"] * 8)
                for rr, a, b in ((8 * g, er + orr, ei + oi), (128 + 8 * g, er - orr, oi - ei)):
                    comps = (a, b - a, a + b) if is_k else (a + b, a, b)
                    for ci, val in enumerate(comps):
                        dst[p, ci, rr:rr + 8, LT(l)] = val
        for l in ls:
            ready.add(("k" if is_k else "x", p, l))

    def stage_x(p, ls):
        force("kv", p)

        def src(l):
            eo = kvv.pop((p, l))
            return (jnp.concatenate([x[0] for x in eo], axis=0), jnp.concatenate([x[1] for x in eo], axis=0))

        fwd(p, ls, src, XS, False)

    def stage_k(p, ls):
        force("kt", p)
        fwd(p, ls, lambda l: (KT[l, pl.ds(p * SB, 128, stride=2), :], KT[l, pl.ds(p * SB + 1, 128, stride=2), :]),
            KS, True)

    ymark = {}
    tdone = {}

    def mac_gen(terms, first, last, g8, l):
        L = LT(l)
        ms = sorted(terms)
        iis = sorted(set(i for m in ms for i in terms[m]))
        Y = {}
        cnt = 0
        for qt in range(4):
            g = 8 * qt + g8
            R = slice(8 * g, 8 * g + 8)
            R2 = slice(SB + 8 * g, SB + 8 * g + 8)
            res = {}
            for c in range(3):
                kc = {}
                acc = {}
                for m in ms:
                    if c == 0:
                        acc[m] = None
                    elif first[m]:
                        acc[m] = res[m, 0]
                    else:
                        acc[m] = res[m, 0] + PS[m, R2 if c == 1 else R, L]
                        cnt += 1
                for i in iis:
                    x = XS[i, c, R, L]
                    for m in ms:
                        if i not in terms[m]:
                            continue
                        a = m - i
                        if a not in kc:
                            kc[a] = KS[a, c, R, L]
                        t = x * kc[a]
                        acc[m] = t if acc[m] is None else (acc[m] - t if c == 2 else acc[m] + t)
                        cnt += 2
                    if cnt >= cfg["G"] and not (c == 2 and i == iis[-1]):
                        yield cnt, [acc[m] for m in ms if acc[m] is not None]
                        cnt = 0
                for m in ms:
                    res[m, c] = acc[m]
            outs = []
            for m in ms:
                re, im = res[m, 2], res[m, 1]
                if not (last[m] and (m + 1 == NP or (m + 1 in ms and last[m + 1]))):
                    PS[m, R, L] = re
                    PS[m, R2, L] = im
                if last[m]:
                    if m > 0:
                        if m - 1 in ms:
                            assert last[m - 1]
                            pr, pi = res[m - 1, 2], res[m - 1, 1]
                        else:
                            pr, pi = PS[m - 1, R, L], PS[m - 1, R2, L]
                        re, im = (re - pi, im + pr) if qt in (0, 3) else (re + pi, im - pr)
                    Y[m, qt] = (re, im)
                outs += [re, im]
            yield cnt + 2 * len(outs), outs
            cnt = 0
        for m in ms:
            if not last[m]:
                continue
            (r0, i0), (r1, i1), (r2, i2), (r3, i3) = (Y[m, qt] for qt in range(4))
            ur0, ui0, vr0, vi0 = r0 + r2, i0 - i2, r0 - r2, i0 + i2
            ur1, ui1, vr1, vi1 = r1 + r3, i1 - i3, r1 - r3, i1 + i3
            ws = (ur0 + ur1, ui0 - ui1, vr0 - vi1, vi0 - vr1, ur0 - ur1, ui0 + ui1, vr0 + vi1, vi0 + vr1)
            for j, w in enumerate(ws):
                YS[m, 64 * j + 8 * g8:64 * j + 8 * g8 + 8, L] = w
            ymark[m, l] = ymark.get((m, l), 0) + 1
            yield 24, list(ws)

    def push_mac(ms, lim=NP):
        for idx in range(8 * NL):
            l, g = idx // 8, idx % 8
            terms, first, last = {}, {}, {}
            for m in ms:
                done = tdone.setdefault((m, idx), set())
                t = [i for i in range(m + 1) if i <= lim and m - i <= lim and i not in done]
                if not t:
                    continue
                for i in t:
                    assert ("x", i, l) in ready and ("k", m - i, l) in ready, (m, i)
                terms[m], first[m] = t, not done
                done.update(t)
                last[m] = len(done) == m + 1
                if last[m] and m > 0 and m - 1 not in ms:
                    assert len(tdone[m - 1, idx]) == m
            if terms:
                Q["mac"].append((min(ms), mac_gen(terms, first, last, g, l)))
        q = Q["mac"]
        head = q[:1] if q and st["cur"] is q[0] else []
        q[:] = head + sorted(q[len(head):], key=lambda e: e[0])

    def ln(x, scale=1.0):
        m = jnp.mean(x, axis=-1, keepdims=True)
        xc = x - m
        ss = jnp.sum(xc * xc, axis=-1, keepdims=True)
        r = jnp.exp(math.log(scale * math.sqrt(D)) - 0.5 * jnp.log(ss + D * EPS))
        return xc * r

    def lq_job(r0):
        xn = ln(qb[r0:r0 + 8, :].astype(f32))
        XN[r0:r0 + 8, :] = xn
        return [xn[:, LT(l)] for l in range(NL)]

    def push_lq(*ps):
        for p in ps:
            for g in range(32):
                Q["lq"].append([0, 34, functools.partial(lq_job, p * SB + 8 * g), p])

    def stage_c(p, ls):
        while any(ymark.get((p, l), 0) < 8 for l in ls):
            finish_mac()
        gm = pltpu.bitcast(gu[...], bf16)
        for l in ls:
            for c in range(4):
                YT[l, pl.ds(p * SB + c, 64, stride=4), :] = jnp.dot(
                    gm[64 * c:64 * c + 64], YS[p, 128 * c:128 * c + 128, LT(l)].astype(bf16),
                    preferred_element_type=f32)
        if ls[-1] != NL - 1:
            return

        def job(r0):
            force("lq", p)
            x = qb[r0:r0 + 8, :].astype(f32)
            h = x + XN[r0:r0 + 8, :] * jnp.concatenate([YT[l, r0:r0 + 8, :] for l in range(NL)], axis=1)
            HR[r0:r0 + 8, :] = h
            hn = ln(h, BETA)
            HN[r0:r0 + 8, :] = hn
            return [hn[:, LT(l)] for l in range(NL)]

        for g in range(32):
            Q["c"].append([cfg["c_delay"] if g == 0 else 0, 42, functools.partial(job, p * SB + 8 * g), p])

    def retile_w1(c0, c1):
        lo, hi = c0 * 128, min(c1 * 128, F)
        w1u[lo // 2:hi // 2, :] = pltpu.bitcast(w1t[lo:hi, :], u32)

    def retile_w2():
        w2u[...] = pltpu.bitcast(w2[...], u32)

    hs, os_ = {}, {}

    def stage_f1(b, nb, c0, c1, save):
        r0 = b * B
        force("c", b // 2)
        hn = cached(("hn", b), lambda: HN[r0:r0 + nb * B, :].astype(bf16))
        b1 = cached("b1", lambda: BETA * b1b[...].astype(f32)[None, :])
        out = {} if save else hs.setdefault(b, {})
        for c in range(c0, c1):
            lo, hi = c * 128, min((c + 1) * 128, F)
            w = pltpu.bitcast(w1u[lo // 2:hi // 2, :], bf16)
            init = linked_init(jnp.broadcast_to(b1[:, lo:hi], (nb * B, hi - lo)), cfg["cap1"] * 8)
            t = lax.dot_general(hn, w, NT, preferred_element_type=f32) + init
            out[c] = t + t * jnp.tanh(t * (KAPPA + t * t))
            if save:
                H1[r0:r0 + nb * B, lo:hi] = out[c]

    def stage_f2(b, nb, l0, l1):
        r0 = b * B
        if b in hs:
            if isinstance(hs[b], dict):
                hs[b] = tuple(jnp.concatenate([hs[b][c] for c in range(k0 // 128, (k1 + 127) // 128)],
                                              axis=1).astype(bf16) for k0, k1 in KG)
        else:
            hs[b] = tuple(H1[r0:r0 + nb * B, k0:k1].astype(bf16) for k0, k1 in KG)
        b2 = cached("b2", lambda: (1.0 / GAMMA) * b2b[...].astype(f32)[None, :])
        out = os_.setdefault(b, [])
        for l in range(l0, l1):
            o = jnp.broadcast_to(b2[:, LT(l)], (nb * B, 128))
            for (k0, k1), hk in zip(KG, hs[b]):
                o = jnp.dot(hk, pltpu.bitcast(w2u[k0 // 2:k1 // 2, LT(l)], bf16), preferred_element_type=f32
                            ) + linked_init(o, cfg["cap2"] * 8 * (k1 - k0) / 512)
            out.append(o)
        if l1 == NL:
            o = jnp.concatenate(os_.pop(b), axis=1)
            hs.pop(b)
            ob[r0:r0 + nb * B, :] = (HR[r0:r0 + nb * B, :] + GAMMA * o).astype(bf16)
            out_copy(b, nb).start()

    ops = dict(hold=lambda v: st.update(hold=v), set=lambda k, v: cfg.update({k: v}), tables=tables,
               kv=push_kv, kt=push_kt, lq=push_lq, x=stage_x, k=stage_k, mac=push_mac, c=stage_c,
               f1=stage_f1, f2=stage_f2, rw1=retile_w1, rw2=retile_w2)

    nreg = len(plan["prog"])
    for ridx, region in enumerate(plan["prog"]):
        @pl.when(pid == ridx)
        def _(region=region, ridx=ridx):
            if ridx > 0:
                st["never"] = lax.broadcasted_iota(jnp.int32, (8, 128), 0) < zs[0]
            st["cache"] = {}
            for step in region:
                if step[0] == "wait":
                    for c in groups[step[1]]:
                        c.wait()
                else:
                    ops[step[0]](*step[1:])
            if Q["mac"] and st["cur"] is Q["mac"][0]:
                finish_mac()
            for name in ("c", "kt", "kv", "lq"):
                while Q[name]:
                    Q[name].pop(0)[2]()
            st["credit"] = 0.0
            assert not hs and not os_ and not kvv
            if ridx == nreg - 1:
                assert not Q["mac"]
                out_copy(0, NB).wait()


def _plan():
    cfg = dict(G=32, cap1=1.6, cap2=2.2, capx=1.6, mul=1.0, maxcredit=40, c_delay=24)
    n1 = 5
    dma = [("s0", ["sk", ("s", 0, 2)]), ("a0", [("kv", 0, 1)]), ("q0", [("q", 0, 1), "small"]),
           ("g1", [("kv", 1, 2)]), ("w1a", [("w1", 0, n1)]), ("w1b", [("q", 1, 2), ("w1", n1, 11)]),
           ("g2", [("skvq", 2, 3)]), ("w2", [("w2", 0, 11)]), ("g3", [("skv", 3, 4)]),
           ("g4", [("q", 3, 4), ("skv", 4, 8)]), ("q4", [("q", 4, 8)])]
    A, Z = (0, 1), (2, 3)
    W = lambda n: [("wait", n)]
    kv = lambda *ps: [("kv", *ps)]
    kt = lambda *ps: [("kt", *ps)]
    lq = lambda *ps: [("lq", *ps)]
    K = lambda p, ls: [("k", p, ls)]
    X = lambda p, ls: [("x", p, ls)]
    C = lambda p: [("c", p, A), ("c", p, Z)]
    M = lambda ms, lim=NP: [("mac", ms, lim)]
    F1 = lambda p, c0, c1: [("f1", 2 * p, 2, c0, c1, False)]
    S1 = lambda p, c0, c1: [("f1", 2 * p, 2, c0, c1, True)]
    F2 = lambda p, l0, l1: [("f2", 2 * p, 2, l0, l1)]
    FC = lambda p: lq(p + 1) + F1(p, 0, 11) + F2(p, 0, 1) + C(p + 1) + F2(p, 1, 4)
    prog = [
        [("tables",)] + W("s0") + kt(0, 1) + K(0, A) + K(0, Z),
        W("a0") + [("hold", True), ("set", "cap1", 2.2), ("set", "capx", 2.2)]
        + kv(0) + K(1, A) + X(0, A) + X(0, Z) + M([0]) + K(1, Z) + C(0)
        + W("q0") + W("g1") + [("hold", False)] + lq(0) + kv(1) + X(1, A) + X(1, Z),
        W("w1a") + [("rw1", 0, n1), ("hold", True)] + M([1]) + S1(0, 0, n1 - 1) + [("c", 1, A)]
        + S1(0, n1 - 1, n1) + [("c", 1, Z)]
        + W("w1b") + [("rw1", n1, 11)] + lq(1) + S1(0, n1, n1 + 2) + [("hold", False)] + S1(0, n1 + 2, 11),
        W("g2") + [("set", "cap1", cfg["cap1"]), ("set", "capx", cfg["capx"])] + kt(2) + kv(2) + lq(2) + M([2], 1)
        + S1(1, 0, 2) + K(2, A) + S1(1, 2, 4) + K(2, Z) + S1(1, 4, 6) + X(2, A) + S1(1, 6, 8) + X(2, Z)
        + S1(1, 8, 11),
        W("w2") + W("g3") + [("rw2",)] + M([2]) + M([3, 4], 2) + F2(0, 0, 2) + C(2) + F2(0, 2, 3)
        + kt(3) + kv(3) + F2(0, 3, 4) + F2(1, 0, 1) + K(3, A) + K(3, Z) + F2(1, 1, 2) + X(3, A) + F2(1, 2, 3)
        + X(3, Z) + F2(1, 3, 4),
        W("g4") + kt(4) + lq(3) + M([3]) + M([4, 5], 3) + F1(2, 0, 3) + K(4, A) + kt(5)
        + F1(2, 3, 4) + K(4, Z) + F1(2, 4, 6) + K(5, A) + kt(6) + F1(2, 6, 7) + K(5, Z) + F1(2, 7, 8) + C(3)
        + kt(7) + kv(4, 5, 6, 7) + F1(2, 8, 9) + K(6, A) + F1(2, 9, 10) + K(6, Z) + F1(2, 10, 11) + K(7, A)
        + F2(2, 0, 1) + K(7, Z) + X(4, A) + F2(2, 1, 2) + X(4, Z) + X(5, A) + F2(2, 2, 3) + X(5, Z) + X(6, A)
        + F2(2, 3, 4) + X(6, Z) + S1(3, 0, 2) + X(7, A) + S1(3, 2, 3) + X(7, Z),
        W("q4") + [("set", "mul", 0.9)] + lq(4) + M([4]) + M([5]) + M([6]) + M([7])
        + S1(3, 3, 11) + F2(3, 0, 1) + C(4) + F2(3, 1, 4) + FC(4) + FC(5) + FC(6)
        + [("f1", 14, 1, 0, 11, False), ("f1", 15, 1, 0, 11, False), ("f2", 14, 1, 0, 4), ("f2", 15, 1, 0, 4)],
    ]
    return dict(dma=dma, prog=prog, cfg=cfg)


@jax.jit
def pallas_sequential_preLN__ssm_conv_h3__dense_activation_gelu__prompt_kernel(
    A_q: jax.Array,
    A_k: jax.Array,
    A_v: jax.Array,
    A_shift_k: jax.Array,
    A_ssm_k: jax.Array,
    A_ssm_D: jax.Array,
    B_x: jax.Array,
    B_w1: jax.Array,
    B_b1: jax.Array,
    B_w2: jax.Array,
    B_b2: jax.Array,
):
    plan = _plan()
    ANY = pl.BlockSpec(memory_space=pl.ANY)
    V = pltpu.VMEM
    scratch = [
        V((S, D), bf16), V((S, D), bf16), V((S, D), bf16), V((D, S), bf16),
        V((F, D), bf16), V((F, D), bf16),
        V((4, D), bf16), V((D,), bf16), V((F,), bf16), V((D,), bf16),
        V((NL, S + 16, 128), f32), V((S, D), bf16),
        V((F // 2, D), u32), V((F // 2, D), u32),
        V((128, 128), u32), V((128, 128), u32), V((128, 128), u32),
        V((NP, 3, SB, D), f32), V((NP, 3, SB, D), f32),
        V((NP, 2 * SB, D), f32), V((NP, 2 * SB, D), f32),
        V((S, D), f32), V((S, D), f32),
        V((4 * SB, F), f32), V((NL, S + 8, 128), f32), V((NL, S + 8, 128), f32),
        V((S, D), f32),
        pltpu.SMEM((1,), jnp.int32),
        pltpu.SemaphoreType.DMA((len(plan["dma"]),)), pltpu.SemaphoreType.DMA((1,)),
    ]
    out = pl.pallas_call(
        functools.partial(_kernel, plan=plan),
        grid=(len(plan["prog"]),),
        in_specs=[ANY] * 10,
        out_specs=ANY,
        out_shape=jax.ShapeDtypeStruct((S, D), bf16),
        scratch_shapes=scratch,
        compiler_params=pltpu.CompilerParams(
            dimension_semantics=("arbitrary",), vmem_limit_bytes=120 * 1024 * 1024,
            disable_semaphore_checks=True, disable_bounds_checks=True),
    )(A_q.reshape(S, D), A_k.reshape(S, D), A_v.reshape(S, D), A_shift_k.T, A_ssm_k, A_ssm_D,
      B_w1.T, B_b1, B_w2, B_b2)
    return out.reshape(1, S, D)
```

```python
import functools
import math

import jax
import jax.numpy as jnp
from jax import lax
import jax.experimental.pallas as pl
import jax.experimental.pallas.tpu as pltpu

S, D, F = 2048, 512, 1376
B = 128
NB = S // B
SB = 256
NP = S // SB
NL = D // 128
NF = (F + 127) // 128
EPS = 1e-5
f32, bf16, u32 = jnp.float32, jnp.bfloat16, jnp.uint32
NT = (((1,), (1,)), ((), ()))
C0 = math.sqrt(2.0 / math.pi)
C1 = C0 * 0.044715
KG = ((0, 512), (512, 1024), (1024, F))
BETA = C1 ** (1.0 / 3.0)
KAPPA = C0 / BETA
GAMMA = 0.5 / BETA


def _kernel(q_hbm, k_hbm, v_hbm, sk_hbm, ssm_hbm, sd_hbm, w1t_hbm, b1_hbm, w2_hbm, b2_hbm,
            o_hbm,
            qb, kb, vb, ssm, w1t, w2, skb, sdb, b1b, b2b, kf, ob,
            w1u, w2u, fe, fo, gu, XS, KS, PS, YS, HR, HN, H1, YT, KT, XN,
            zs, isem, osem, *, plan):
    cfg = dict(plan["cfg"])
    pid = pl.program_id(0)

    groups = {}
    for gi, (name, spec) in enumerate(plan["dma"]):
        cp = lambda src, dst: pltpu.make_async_copy(src, dst, isem.at[gi])
        cs = []
        for item in spec:
            if item == "sk":
                cs += [cp(sk_hbm, skb), cp(sd_hbm, sdb)]
            elif item == "small":
                cs += [cp(b1_hbm, b1b), cp(b2_hbm, b2b)]
            elif item[0] in ("w1", "w2"):
                src, dst = (w1t_hbm, w1t) if item[0] == "w1" else (w2_hbm, w2)
                r = pl.ds(item[1] * 128, min(item[2] * 128, F) - item[1] * 128)
                cs += [cp(src.at[r], dst.at[r])]
            else:
                r = pl.ds(item[1] * SB, (item[2] - item[1]) * SB)
                for ch in item[0]:
                    if ch == "s":
                        cs.append(cp(ssm_hbm.at[:, r], ssm.at[:, r]))
                    else:
                        src, dst = dict(k=(k_hbm, kb), v=(v_hbm, vb), q=(q_hbm, qb))[ch]
                        cs.append(cp(src.at[r], dst.at[r]))
        groups[name] = cs

    def out_copy(b, nb):
        r = pl.ds(b * B, nb * B)
        return pltpu.make_async_copy(ob.at[r], o_hbm.at[r], osem.at[0])

    Q = dict(c=[], kt=[], kv=[], lq=[], mac=[])
    st = dict(credit=0.0, never=None, cache={}, hold=False, cur=None)

    def cached(key, fn):
        if key not in st["cache"]:
            st["cache"][key] = fn()
        return st["cache"][key]

    def LT(l):
        return slice(l * 128, (l + 1) * 128)

    def tables():
        for cs in groups.values():
            for c in cs:
                c.start()
        zs[0] = 0

        def cosn(n, scale):
            n = jnp.abs((n & 1023) - 512)
            x = (n - 256).astype(f32) * (2.0 * math.pi / 1024)
            x2 = x * x
            p = -1.0 / 39916800.0
            for cf in (1.0 / 362880.0, -1.0 / 5040.0, 1.0 / 120.0, -1.0 / 6.0, 1.0):
                p = p * x2 + cf
            return p * (x * scale)

        r = lax.broadcasted_iota(jnp.int32, (256, 128), 0)
        c = lax.broadcasted_iota(jnp.int32, (256, 128), 1)
        slot_ = ((r >> 5) << 4) + (r & 15)
        odd = jnp.where(slot_ < 64, 4 * slot_ + 1, 511 - 4 * slot_)
        ne = odd * (2 * c) + ((r & 16) << 4)
        fe[...] = pltpu.bitcast(cosn(ne, 1.0).astype(bf16), u32)
        fo[...] = pltpu.bitcast(cosn(ne + odd, 1.0).astype(bf16), u32)
        j = 4 * (r & 63) + (r >> 6)
        gu[...] = pltpu.bitcast(cosn((4 * (c & 63) + 1) * j + ((c & 64) << 2), 1.0 / 256).astype(bf16), u32)
        for l in range(NL):
            kf[l, 0:8, :] = jnp.zeros((8, 128), f32)

    def take(cap):
        if st["never"] is None:
            return None
        st["credit"] = min(st["credit"] + cap * cfg["mul"], cfg["maxcredit"])
        deps = []
        for name in ("c", "kt", "kv", "lq"):
            q = Q[name]
            if name == "c" and st["hold"]:
                continue
            if q and q[0][0] > 0:
                q[0][0] -= 1
                continue
            while q and q[0][0] == 0 and st["credit"] > 0:
                j = q.pop(0)
                st["credit"] -= j[1]
                deps += j[2]()
        q = Q["mac"]
        while q and st["credit"] > 0:
            st["cur"] = q[0]
            nxt = next(q[0][1], None)
            if nxt is None:
                q.pop(0)
                continue
            st["credit"] -= nxt[0]
            deps += nxt[1]
        return functools.reduce(lambda x, y: x + y, deps) if deps else None

    def tie(piece, d):
        w = piece.shape[1]
        if w == 128:
            return lax.select(st["never"], d, piece)
        return lax.select(cached(("never", w), lambda: st["never"][:, :w]), d[:, :w], piece)

    def linked_init(init, cap):
        parts, start = [], 0
        for r in range(0, init.shape[0], 8):
            d = take(cap)
            if d is not None:
                if start < r:
                    parts.append(init[start:r])
                parts.append(tie(init[r:r + 8], d))
                start = r + 8
        if not parts:
            return init
        if start < init.shape[0]:
            parts.append(init[start:])
        return jnp.concatenate(parts, axis=0)

    def force(name, tag):
        while any(j[3] == tag for j in Q[name]):
            Q[name].pop(0)[2]()

    def finish_mac():
        for _ in Q["mac"].pop(0)[1]:
            pass

    kvv = {}

    def ku_job(r0):
        kall = kb[r0:r0 + 16, :].astype(f32)
        for l in range(NL):
            kf[l, 8 + r0:24 + r0, :] = kall[:, LT(l)]
        return [kall[8:16, LT(NL - 1)]]

    def kv_job(p, g, ls):
        r0 = p * SB + 16 * g
        sk = cached("sk", lambda: skb[...].astype(f32))
        outs = []
        for l in ls:
            vw = pltpu.bitcast(vb[r0:r0 + 16, LT(l)], u32)
            ve = pltpu.bitcast(vw << 16, f32)
            vo = pltpu.bitcast(vw & jnp.uint32(0xFFFF0000), f32)
            a = {o: kf[l, pl.ds(8 + r0 + o, 8, stride=2), :] for o in range(-3, 2)}
            w = [sk[t:t + 1, LT(l)] for t in range(4)]
            e = (a[0] * w[0] + a[-1] * w[1] + a[-2] * w[2] + a[-3] * w[3]) * ve
            o = (a[1] * w[0] + a[0] * w[1] + a[-1] * w[2] + a[-2] * w[3]) * vo
            kvv.setdefault((p, l), []).append((e, o))
            outs += [e, o]
        return outs

    def push_kv(*ps):
        for p in ps:
            for g in range(16):
                Q["kv"].append([0, 20, functools.partial(ku_job, p * SB + 16 * g), p])
        for p in ps:
            for g in range(16):
                for ls in ((0, 1), (2, 3)):
                    Q["kv"].append([0, 56, functools.partial(kv_job, p, g, ls), p])

    def kt_job(t0, l):
        t = jnp.transpose(ssm[LT(l), t0:t0 + 128].astype(f32))
        KT[l, t0:t0 + 128, :] = t
        return [t[120:128]]

    def push_kt(*ps):
        for p in ps:
            for l in range(NL):
                for h in range(2):
                    Q["kt"].append([0, 60, functools.partial(kt_job, p * SB + h * 128, l), p])

    ready = set()

    def fwd(p, ls, src, dst, is_k):
        fem, fom = pltpu.bitcast(fe[...], bf16), pltpu.bitcast(fo[...], bf16)
        res = {}
        for l in ls:
            ze, zo = src(l)
            res[l] = (jnp.dot(fem, ze.astype(bf16), preferred_element_type=f32),
                      jnp.dot(fom, zo.astype(bf16), preferred_element_type=f32))
        L = slice(128 * ls[0], 128 * ls[0] + 256)
        e = jnp.concatenate([res[l][0] for l in ls], axis=1)
        o = jnp.concatenate([res[l][1] for l in ls], axis=1)
        for g in range(16):
            r0 = (g // 2) * 32 + (g % 2) * 8
            er, ei, orr, oi = e[r0:r0 + 8], e[r0 + 16:r0 + 24], o[r0:r0 + 8], o[r0 + 16:r0 + 24]
            if is_k and p == 0:
                er = er + cached("sd", lambda: sdb[...].astype(f32)[None, :])[:, L]
            ds = [take(cfg["capx"] * 8) for _ in range(2)]
            if any(d is not None for d in ds):
                er = jnp.concatenate([er[:, LT(j)] if d is None else tie(er[:, LT(j)], d)
                                      for j, d in enumerate(ds)], axis=1)
            for rr, a, b in ((8 * g, er + orr, ei + oi), (128 + 8 * g, er - orr, oi - ei)):
                comps = (a, b - a, a + b) if is_k else (a + b, a, b)
                for ci, val in enumerate(comps):
                    dst[p, ci, rr:rr + 8, L] = val
        for l in ls:
            ready.add(("k" if is_k else "x", p, l))

    def stage_x(p, ls):
        force("kv", p)

        def src(l):
            eo = kvv.pop((p, l))
            return (jnp.concatenate([x[0] for x in eo], axis=0), jnp.concatenate([x[1] for x in eo], axis=0))

        fwd(p, ls, src, XS, False)

    def stage_k(p, ls):
        force("kt", p)
        fwd(p, ls, lambda l: (KT[l, pl.ds(p * SB, 128, stride=2), :], KT[l, pl.ds(p * SB + 1, 128, stride=2), :]),
            KS, True)

    ymark = {}
    tdone = {}

    def mac_gen(terms, first, last, g8, l):
        L = LT(l)
        ms = sorted(terms)
        iis = sorted(set(i for m in ms for i in terms[m]))
        Y = {}
        cnt = 0
        for qt in range(4):
            g = 8 * qt + g8
            R = slice(8 * g, 8 * g + 8)
            R2 = slice(SB + 8 * g, SB + 8 * g + 8)
            res = {}
            for c in range(3):
                kc = {}
                acc = {}
                for m in ms:
                    if c == 0:
                        acc[m] = None
                    elif first[m]:
                        acc[m] = res[m, 0]
                    else:
                        acc[m] = res[m, 0] + PS[m, R2 if c == 1 else R, L]
                        cnt += 1
                for i in iis:
                    x = XS[i, c, R, L]
                    for m in ms:
                        if i not in terms[m]:
                            continue
                        a = m - i
                        if a not in kc:
                            kc[a] = KS[a, c, R, L]
                        t = x * kc[a]
                        acc[m] = t if acc[m] is None else (acc[m] - t if c == 2 else acc[m] + t)
                        cnt += 2
                    if cnt >= cfg["G"] and not (c == 2 and i == iis[-1]):
                        yield cnt, [acc[m] for m in ms if acc[m] is not None]
                        cnt = 0
                for m in ms:
                    res[m, c] = acc[m]
            outs = []
            for m in ms:
                re, im = res[m, 2], res[m, 1]
                if not (last[m] and (m + 1 == NP or (m + 1 in ms and last[m + 1]))):
                    PS[m, R, L] = re
                    PS[m, R2, L] = im
                if last[m]:
                    if m > 0:
                        if m - 1 in ms:
                            assert last[m - 1]
                            pr, pi = res[m - 1, 2], res[m - 1, 1]
                        else:
                            pr, pi = PS[m - 1, R, L], PS[m - 1, R2, L]
                        re, im = (re - pi, im + pr) if qt in (0, 3) else (re + pi, im - pr)
                    Y[m, qt] = (re, im)
                outs += [re, im]
            yield cnt + 2 * len(outs), outs
            cnt = 0
        for m in ms:
            if not last[m]:
                continue
            (r0, i0), (r1, i1), (r2, i2), (r3, i3) = (Y[m, qt] for qt in range(4))
            ur0, ui0, vr0, vi0 = r0 + r2, i0 - i2, r0 - r2, i0 + i2
            ur1, ui1, vr1, vi1 = r1 + r3, i1 - i3, r1 - r3, i1 + i3
            ws = (ur0 + ur1, ui0 - ui1, vr0 - vi1, vi0 - vr1, ur0 - ur1, ui0 + ui1, vr0 + vi1, vi0 + vr1)
            for j, w in enumerate(ws):
                YS[m, 64 * j + 8 * g8:64 * j + 8 * g8 + 8, L] = w
            ymark[m, l] = ymark.get((m, l), 0) + 1
            yield 24, list(ws)

    def push_mac(ms, lim=NP):
        for idx in range(8 * NL):
            l, g = idx // 8, idx % 8
            terms, first, last = {}, {}, {}
            for m in ms:
                done = tdone.setdefault((m, idx), set())
                t = [i for i in range(m + 1) if i <= lim and m - i <= lim and i not in done]
                if not t:
                    continue
                for i in t:
                    assert ("x", i, l) in ready and ("k", m - i, l) in ready, (m, i)
                terms[m], first[m] = t, not done
                done.update(t)
                last[m] = len(done) == m + 1
                if last[m] and m > 0 and m - 1 not in ms:
                    assert len(tdone[m - 1, idx]) == m
            if terms:
                Q["mac"].append((min(ms), mac_gen(terms, first, last, g, l)))
        q = Q["mac"]
        head = q[:1] if q and st["cur"] is q[0] else []
        q[:] = head + sorted(q[len(head):], key=lambda e: e[0])

    def ln(x, scale=1.0):
        m = jnp.mean(x, axis=-1, keepdims=True)
        xc = x - m
        ss = jnp.sum(xc * xc, axis=-1, keepdims=True)
        r = jnp.exp(math.log(scale * math.sqrt(D)) - 0.5 * jnp.log(ss + D * EPS))
        return xc * r

    def lq_job(r0):
        xn = ln(qb[r0:r0 + 8, :].astype(f32))
        XN[r0:r0 + 8, :] = xn
        return [xn[:, LT(l)] for l in range(NL)]

    def push_lq(*ps):
        for p in ps:
            for g in range(32):
                Q["lq"].append([0, 34, functools.partial(lq_job, p * SB + 8 * g), p])

    def stage_c(p, ls):
        while any(ymark.get((p, l), 0) < 8 for l in ls):
            finish_mac()
        gm = pltpu.bitcast(gu[...], bf16)
        for l in ls:
            for c in range(4):
                YT[l, pl.ds(p * SB + c, 64, stride=4), :] = jnp.dot(
                    gm[64 * c:64 * c + 64], YS[p, 128 * c:128 * c + 128, LT(l)].astype(bf16),
                    preferred_element_type=f32)
        if ls[-1] != NL - 1:
            return

        def job(r0):
            force("lq", p)
            x = qb[r0:r0 + 8, :].astype(f32)
            h = x + XN[r0:r0 + 8, :] * jnp.concatenate([YT[l, r0:r0 + 8, :] for l in range(NL)], axis=1)
            HR[r0:r0 + 8, :] = h
            hn = ln(h, BETA)
            HN[r0:r0 + 8, :] = hn
            return [hn[:, LT(l)] for l in range(NL)]

        for g in range(32):
            Q["c"].append([cfg["c_delay"] if g == 0 else 0, 42, functools.partial(job, p * SB + 8 * g), p])

    def retile_w1(c0, c1):
        lo, hi = c0 * 128, min(c1 * 128, F)
        w1u[lo // 2:hi // 2, :] = pltpu.bitcast(w1t[lo:hi, :], u32)

    def retile_w2():
        w2u[...] = pltpu.bitcast(w2[...], u32)

    hs, os_ = {}, {}

    def stage_f1(b, nb, c0, c1, save):
        r0 = b * B
        force("c", b // 2)
        hn = cached(("hn", b), lambda: HN[r0:r0 + nb * B, :].astype(bf16))
        b1 = cached("b1", lambda: BETA * b1b[...].astype(f32)[None, :])
        out = {} if save else hs.setdefault(b, {})
        for c in range(c0, c1):
            lo, hi = c * 128, min((c + 1) * 128, F)
            w = pltpu.bitcast(w1u[lo // 2:hi // 2, :], bf16)
            init = linked_init(jnp.broadcast_to(b1[:, lo:hi], (nb * B, hi - lo)), cfg["cap1"] * 8)
            t = lax.dot_general(hn, w, NT, preferred_element_type=f32) + init
            out[c] = t + t * jnp.tanh(t * (KAPPA + t * t))
            if save:
                H1[r0:r0 + nb * B, lo:hi] = out[c]

    def stage_f2(b, nb, l0, l1):
        r0 = b * B
        if b in hs:
            if isinstance(hs[b], dict):
                hs[b] = tuple(jnp.concatenate([hs[b][c] for c in range(k0 // 128, (k1 + 127) // 128)],
                                              axis=1).astype(bf16) for k0, k1 in KG)
        else:
            hs[b] = tuple(H1[r0:r0 + nb * B, k0:k1].astype(bf16) for k0, k1 in KG)
        b2 = cached("b2", lambda: (1.0 / GAMMA) * b2b[...].astype(f32)[None, :])
        out = os_.setdefault(b, [])
        for l in range(l0, l1):
            o = jnp.broadcast_to(b2[:, LT(l)], (nb * B, 128))
            for (k0, k1), hk in zip(KG, hs[b]):
                o = jnp.dot(hk, pltpu.bitcast(w2u[k0 // 2:k1 // 2, LT(l)], bf16), preferred_element_type=f32
                            ) + linked_init(o, cfg["cap2"] * 8 * (k1 - k0) / 512)
            out.append(o)
        if l1 == NL:
            o = jnp.concatenate(os_.pop(b), axis=1)
            hs.pop(b)
            ob[r0:r0 + nb * B, :] = (HR[r0:r0 + nb * B, :] + GAMMA * o).astype(bf16)
            out_copy(b, nb).start()

    ops = dict(hold=lambda v: st.update(hold=v), set=lambda k, v: cfg.update({k: v}), tables=tables,
               kv=push_kv, kt=push_kt, lq=push_lq, x=stage_x, k=stage_k, mac=push_mac, c=stage_c,
               f1=stage_f1, f2=stage_f2, rw1=retile_w1, rw2=retile_w2)

    nreg = len(plan["prog"])
    for ridx, region in enumerate(plan["prog"]):
        @pl.when(pid == ridx)
        def _(region=region, ridx=ridx):
            if ridx > 0:
                st["never"] = lax.broadcasted_iota(jnp.int32, (8, 128), 0) < zs[0]
            st["cache"] = {}
            for step in region:
                if step[0] == "wait":
                    for c in groups[step[1]]:
                        c.wait()
                else:
                    ops[step[0]](*step[1:])
            if Q["mac"] and st["cur"] is Q["mac"][0]:
                finish_mac()
            for name in ("c", "kt", "kv", "lq"):
                while Q[name]:
                    Q[name].pop(0)[2]()
            st["credit"] = 0.0
            assert not hs and not os_ and not kvv
            if ridx == nreg - 1:
                assert not Q["mac"]
                out_copy(0, NB).wait()


def _plan():
    cfg = dict(G=32, cap1=1.6, cap2=2.2, capx=1.6, mul=1.0, maxcredit=40, c_delay=24)
    n1 = 5
    dma = [("s0", ["sk", ("s", 0, 2)]), ("a0", [("kv", 0, 1)]), ("q0", [("q", 0, 1), "small"]),
           ("g1", [("kv", 1, 2)]), ("w1a", [("w1", 0, n1)]), ("w1b", [("q", 1, 2), ("w1", n1, 11)]),
           ("g2", [("skvq", 2, 3)]), ("w2", [("w2", 0, 11)]), ("g3", [("skv", 3, 4)]),
           ("g4", [("q", 3, 4), ("skv", 4, 8)]), ("q4", [("q", 4, 8)])]
    A, Z = (0, 1), (2, 3)
    W = lambda n: [("wait", n)]
    kv = lambda *ps: [("kv", *ps)]
    kt = lambda *ps: [("kt", *ps)]
    lq = lambda *ps: [("lq", *ps)]
    K = lambda p, ls: [("k", p, ls)]
    X = lambda p, ls: [("x", p, ls)]
    C = lambda p: [("c", p, A), ("c", p, Z)]
    M = lambda ms, lim=NP: [("mac", ms, lim)]
    F1 = lambda p, c0, c1: [("f1", 2 * p, 2, c0, c1, False)]
    S1 = lambda p, c0, c1: [("f1", 2 * p, 2, c0, c1, True)]
    F2 = lambda p, l0, l1: [("f2", 2 * p, 2, l0, l1)]
    FC = lambda p: lq(p + 1) + F1(p, 0, 11) + F2(p, 0, 1) + C(p + 1) + F2(p, 1, 4)
    prog = [
        [("tables",)] + W("s0") + kt(0, 1) + K(0, A) + K(0, Z),
        W("a0") + [("hold", True), ("set", "cap1", 2.2), ("set", "capx", 2.2)]
        + kv(0) + K(1, A) + X(0, A) + X(0, Z) + M([0]) + K(1, Z) + C(0)
        + W("q0") + W("g1") + [("hold", False)] + lq(0) + kv(1) + X(1, A) + X(1, Z),
        W("w1a") + [("rw1", 0, n1), ("hold", True)] + M([1]) + S1(0, 0, n1 - 1) + [("c", 1, A)]
        + S1(0, n1 - 1, n1) + [("c", 1, Z)]
        + W("w1b") + [("rw1", n1, 11)] + lq(1) + S1(0, n1, n1 + 2) + [("hold", False)] + S1(0, n1 + 2, 11),
        W("g2") + [("set", "cap1", cfg["cap1"]), ("set", "capx", cfg["capx"])] + kt(2) + kv(2) + lq(2) + M([2], 1)
        + S1(1, 0, 2) + K(2, A) + S1(1, 2, 4) + K(2, Z) + S1(1, 4, 6) + X(2, A) + S1(1, 6, 8) + X(2, Z)
        + S1(1, 8, 11),
        W("w2") + W("g3") + [("rw2",)] + M([2]) + M([3, 4], 2) + F2(0, 0, 2) + C(2) + F2(0, 2, 3)
        + kt(3) + kv(3) + F2(0, 3, 4) + F2(1, 0, 1) + K(3, A) + K(3, Z) + F2(1, 1, 2) + X(3, A) + F2(1, 2, 3)
        + X(3, Z) + F2(1, 3, 4),
        W("g4") + kt(4) + lq(3) + M([3]) + M([4, 5], 3) + F1(2, 0, 3) + K(4, A) + kt(5)
        + F1(2, 3, 4) + K(4, Z) + F1(2, 4, 6) + K(5, A) + kt(6) + F1(2, 6, 7) + K(5, Z) + F1(2, 7, 8) + C(3)
        + kt(7) + kv(4, 5, 6, 7) + F1(2, 8, 9) + K(6, A) + F1(2, 9, 10) + K(6, Z) + F1(2, 10, 11) + K(7, A)
        + F2(2, 0, 1) + K(7, Z) + X(4, A) + F2(2, 1, 2) + X(4, Z) + X(5, A) + F2(2, 2, 3) + X(5, Z) + X(6, A)
        + F2(2, 3, 4) + X(6, Z) + S1(3, 0, 2) + X(7, A) + S1(3, 2, 3) + X(7, Z),
        W("q4") + [("set", "mul", 0.9)] + lq(4) + M([4]) + M([5]) + M([6]) + M([7])
        + S1(3, 3, 11) + F2(3, 0, 1) + C(4) + F2(3, 1, 4) + FC(4) + FC(5) + FC(6)
        + [("f1", 14, 1, 0, 11, False), ("f1", 15, 1, 0, 11, False), ("f2", 14, 1, 0, 4), ("f2", 15, 1, 0, 4)],
    ]
    return dict(dma=dma, prog=prog, cfg=cfg)


@jax.jit
def pallas_sequential_preLN__ssm_conv_h3__dense_activation_gelu__prompt_kernel(
    A_q: jax.Array,
    A_k: jax.Array,
    A_v: jax.Array,
    A_shift_k: jax.Array,
    A_ssm_k: jax.Array,
    A_ssm_D: jax.Array,
    B_x: jax.Array,
    B_w1: jax.Array,
    B_b1: jax.Array,
    B_w2: jax.Array,
    B_b2: jax.Array,
):
    plan = _plan()
    ANY = pl.BlockSpec(memory_space=pl.ANY)
    V = pltpu.VMEM
    scratch = [
        V((S, D), bf16), V((S, D), bf16), V((S, D), bf16), V((D, S), bf16),
        V((F, D), bf16), V((F, D), bf16),
        V((4, D), bf16), V((D,), bf16), V((F,), bf16), V((D,), bf16),
        V((NL, S + 16, 128), f32), V((S, D), bf16),
        V((F // 2, D), u32), V((F // 2, D), u32),
        V((128, 128), u32), V((128, 128), u32), V((128, 128), u32),
        V((NP, 3, SB, D), f32), V((NP, 3, SB, D), f32),
        V((NP, 2 * SB, D), f32), V((NP, 2 * SB, D), f32),
        V((S, D), f32), V((S, D), f32),
        V((4 * SB, F), f32), V((NL, S + 8, 128), f32), V((NL, S + 8, 128), f32),
        V((S, D), f32),
        pltpu.SMEM((1,), jnp.int32),
        pltpu.SemaphoreType.DMA((len(plan["dma"]),)), pltpu.SemaphoreType.DMA((1,)),
    ]
    out = pl.pallas_call(
        functools.partial(_kernel, plan=plan),
        grid=(len(plan["prog"]),),
        in_specs=[ANY] * 10,
        out_specs=ANY,
        out_shape=jax.ShapeDtypeStruct((S, D), bf16),
        scratch_shapes=scratch,
        compiler_params=pltpu.CompilerParams(
            dimension_semantics=("arbitrary",), vmem_limit_bytes=120 * 1024 * 1024,
            disable_semaphore_checks=True, disable_bounds_checks=True),
    )(A_q.reshape(S, D), A_k.reshape(S, D), A_v.reshape(S, D), A_shift_k.T, A_ssm_k, A_ssm_D,
      B_w1.T, B_b1, B_w2, B_b2)
    return out.reshape(1, S, D)
```

```python
import functools
import math

import jax
import jax.numpy as jnp
from jax import lax
import jax.experimental.pallas as pl
import jax.experimental.pallas.tpu as pltpu

S, D, F = 2048, 512, 1376
B = 128
NB = S // B
SB = 256
NP = S // SB
NL = D // 128
NF = (F + 127) // 128
EPS = 1e-5
f32, bf16, u32 = jnp.float32, jnp.bfloat16, jnp.uint32
NT = (((1,), (1,)), ((), ()))
C0 = math.sqrt(2.0 / math.pi)
C1 = C0 * 0.044715
KG = ((0, 512), (512, 1024), (1024, F))
BETA = C1 ** (1.0 / 3.0)
KAPPA = C0 / BETA
GAMMA = 0.5 / BETA


def _kernel(q_hbm, k_hbm, v_hbm, sk_hbm, ssm_hbm, sd_hbm, w1t_hbm, b1_hbm, w2_hbm, b2_hbm,
            o_hbm,
            qb, kb, vb, ssm, w1t, w2, skb, sdb, b1b, b2b, kf, ob,
            w1u, w2u, fe, fo, gu, XS, KS, PS, YS, HR, HN, H1, YT, KT, XN,
            zs, isem, osem, *, plan):
    cfg = dict(plan["cfg"])
    pid = pl.program_id(0)

    groups = {}
    for gi, (name, spec) in enumerate(plan["dma"]):
        cp = lambda src, dst: pltpu.make_async_copy(src, dst, isem.at[gi])
        cs = []
        for item in spec:
            if item == "sk":
                cs += [cp(sk_hbm, skb), cp(sd_hbm, sdb)]
            elif item == "small":
                cs += [cp(b1_hbm, b1b), cp(b2_hbm, b2b)]
            elif item[0] in ("w1", "w2"):
                src, dst = (w1t_hbm, w1t) if item[0] == "w1" else (w2_hbm, w2)
                r = pl.ds(item[1] * 128, min(item[2] * 128, F) - item[1] * 128)
                cs += [cp(src.at[r], dst.at[r])]
            else:
                r = pl.ds(item[1] * SB, (item[2] - item[1]) * SB)
                for ch in item[0]:
                    if ch == "s":
                        cs.append(cp(ssm_hbm.at[:, r], ssm.at[:, r]))
                    else:
                        src, dst = dict(k=(k_hbm, kb), v=(v_hbm, vb), q=(q_hbm, qb))[ch]
                        cs.append(cp(src.at[r], dst.at[r]))
        groups[name] = cs

    def out_copy(b, nb):
        r = pl.ds(b * B, nb * B)
        return pltpu.make_async_copy(ob.at[r], o_hbm.at[r], osem.at[0])

    Q = dict(c=[], kt=[], kv=[], lq=[], mac=[])
    st = dict(credit=0.0, never=None, cache={}, hold=False, cur=None)

    def cached(key, fn):
        if key not in st["cache"]:
            st["cache"][key] = fn()
        return st["cache"][key]

    def LT(l):
        return slice(l * 128, (l + 1) * 128)

    def tables():
        for cs in groups.values():
            for c in cs:
                c.start()
        zs[0] = 0

        def cosn(n, scale):
            n = jnp.abs((n & 1023) - 512)
            x = (n - 256).astype(f32) * (2.0 * math.pi / 1024)
            x2 = x * x
            p = -1.0 / 39916800.0
            for cf in (1.0 / 362880.0, -1.0 / 5040.0, 1.0 / 120.0, -1.0 / 6.0, 1.0):
                p = p * x2 + cf
            return p * (x * scale)

        r = lax.broadcasted_iota(jnp.int32, (256, 128), 0)
        c = lax.broadcasted_iota(jnp.int32, (256, 128), 1)
        slot_ = ((r >> 5) << 4) + (r & 15)
        odd = jnp.where(slot_ < 64, 4 * slot_ + 1, 511 - 4 * slot_)
        ne = odd * (2 * c) + ((r & 16) << 4)
        fe[...] = pltpu.bitcast(cosn(ne, 1.0).astype(bf16), u32)
        fo[...] = pltpu.bitcast(cosn(ne + odd, 1.0).astype(bf16), u32)
        j = 4 * (r & 63) + (r >> 6)
        gu[...] = pltpu.bitcast(cosn((4 * (c & 63) + 1) * j + ((c & 64) << 2), 1.0 / 256).astype(bf16), u32)
        for l in range(NL):
            kf[l, 0:8, :] = jnp.zeros((8, 128), f32)

    def take(cap):
        if st["never"] is None:
            return None
        st["credit"] = min(st["credit"] + cap * cfg["mul"], cfg["maxcredit"])
        deps = []
        for name in ("c", "kt", "kv", "lq"):
            q = Q[name]
            if name == "c" and st["hold"]:
                continue
            if q and q[0][0] > 0:
                q[0][0] -= 1
                continue
            while q and q[0][0] == 0 and st["credit"] > 0:
                j = q.pop(0)
                st["credit"] -= j[1]
                deps += j[2]()
        q = Q["mac"]
        while q and st["credit"] > 0:
            st["cur"] = q[0]
            nxt = next(q[0][1], None)
            if nxt is None:
                q.pop(0)
                continue
            st["credit"] -= nxt[0]
            deps += nxt[1]
        return functools.reduce(lambda x, y: x + y, deps) if deps else None

    def tie(piece, d):
        w = piece.shape[1]
        if w == 128:
            return lax.select(st["never"], d, piece)
        return lax.select(cached(("never", w), lambda: st["never"][:, :w]), d[:, :w], piece)

    def linked_init(init, cap):
        parts, start = [], 0
        for r in range(0, init.shape[0], 8):
            d = take(cap)
            if d is not None:
                if start < r:
                    parts.append(init[start:r])
                parts.append(tie(init[r:r + 8], d))
                start = r + 8
        if not parts:
            return init
        if start < init.shape[0]:
            parts.append(init[start:])
        return jnp.concatenate(parts, axis=0)

    def force(name, tag):
        while any(j[3] == tag for j in Q[name]):
            Q[name].pop(0)[2]()

    def finish_mac():
        for _ in Q["mac"].pop(0)[1]:
            pass

    kvv = {}

    def ku_job(r0):
        kall = kb[r0:r0 + 16, :].astype(f32)
        for l in range(NL):
            kf[l, 8 + r0:24 + r0, :] = kall[:, LT(l)]
        return [kall[8:16, LT(NL - 1)]]

    def kv_job(p, g, ls):
        r0 = p * SB + 16 * g
        sk = cached("sk", lambda: skb[...].astype(f32))
        outs = []
        for l in ls:
            vw = pltpu.bitcast(vb[r0:r0 + 16, LT(l)], u32)
            ve = pltpu.bitcast(vw << 16, f32)
            vo = pltpu.bitcast(vw & jnp.uint32(0xFFFF0000), f32)
            a = {o: kf[l, pl.ds(8 + r0 + o, 8, stride=2), :] for o in range(-3, 2)}
            w = [sk[t:t + 1, LT(l)] for t in range(4)]
            e = (a[0] * w[0] + a[-1] * w[1] + a[-2] * w[2] + a[-3] * w[3]) * ve
            o = (a[1] * w[0] + a[0] * w[1] + a[-1] * w[2] + a[-2] * w[3]) * vo
            kvv.setdefault((p, l), []).append((e, o))
            outs += [e, o]
        return outs

    def push_kv(*ps):
        for p in ps:
            for g in range(16):
                Q["kv"].append([0, 20, functools.partial(ku_job, p * SB + 16 * g), p])
        for p in ps:
            for g in range(16):
                for ls in ((0, 1), (2, 3)):
                    Q["kv"].append([0, 56, functools.partial(kv_job, p, g, ls), p])

    def kt_job(t0, l):
        t = jnp.transpose(ssm[LT(l), t0:t0 + 128].astype(f32))
        KT[l, t0:t0 + 128, :] = t
        return [t[120:128]]

    def push_kt(*ps):
        for p in ps:
            for l in range(NL):
                for h in range(2):
                    Q["kt"].append([0, 60, functools.partial(kt_job, p * SB + h * 128, l), p])

    ready = set()

    def fwd(p, ls, src, dst, is_k):
        fem, fom = pltpu.bitcast(fe[...], bf16), pltpu.bitcast(fo[...], bf16)
        res = {}
        for l in ls:
            ze, zo = src(l)
            res[l] = (jnp.dot(fem, ze.astype(bf16), preferred_element_type=f32),
                      jnp.dot(fom, zo.astype(bf16), preferred_element_type=f32))
        L = slice(128 * ls[0], 128 * ls[0] + 256)
        e = jnp.concatenate([res[l][0] for l in ls], axis=1)
        o = jnp.concatenate([res[l][1] for l in ls], axis=1)
        for g in range(16):
            r0 = (g // 2) * 32 + (g % 2) * 8
            er, ei, orr, oi = e[r0:r0 + 8], e[r0 + 16:r0 + 24], o[r0:r0 + 8], o[r0 + 16:r0 + 24]
            if is_k and p == 0:
                er = er + cached("sd", lambda: sdb[...].astype(f32)[None, :])[:, L]
            ds = [take(cfg["capx"] * 8) for _ in range(2)]
            if any(d is not None for d in ds):
                er = jnp.concatenate([er[:, LT(j)] if d is None else tie(er[:, LT(j)], d)
                                      for j, d in enumerate(ds)], axis=1)
            for rr, a, b in ((8 * g, er + orr, ei + oi), (128 + 8 * g, er - orr, oi - ei)):
                comps = (a, b - a, a + b) if is_k else (a + b, a, b)
                for ci, val in enumerate(comps):
                    dst[p, ci, rr:rr + 8, L] = val
        for l in ls:
            ready.add(("k" if is_k else "x", p, l))

    def stage_x(p, ls):
        force("kv", p)

        def src(l):
            eo = kvv.pop((p, l))
            return (jnp.concatenate([x[0] for x in eo], axis=0), jnp.concatenate([x[1] for x in eo], axis=0))

        fwd(p, ls, src, XS, False)

    def stage_k(p, ls):
        force("kt", p)
        fwd(p, ls, lambda l: (KT[l, pl.ds(p * SB, 128, stride=2), :], KT[l, pl.ds(p * SB + 1, 128, stride=2), :]),
            KS, True)

    ymark = {}
    tdone = {}

    def mac_gen(terms, first, last, g8, l):
        L = LT(l)
        ms = sorted(terms)
        iis = sorted(set(i for m in ms for i in terms[m]))
        Y = {}
        cnt = 0
        for qt in range(4):
            g = 8 * qt + g8
            R = slice(8 * g, 8 * g + 8)
            R2 = slice(SB + 8 * g, SB + 8 * g + 8)
            res = {}
            for c in range(3):
                kc = {}
                acc = {}
                for m in ms:
                    if c == 0:
                        acc[m] = None
                    elif first[m]:
                        acc[m] = res[m, 0]
                    else:
                        acc[m] = res[m, 0] + PS[m, R2 if c == 1 else R, L]
                        cnt += 1
                for i in iis:
                    x = XS[i, c, R, L]
                    for m in ms:
                        if i not in terms[m]:
                            continue
                        a = m - i
                        if a not in kc:
                            kc[a] = KS[a, c, R, L]
                        t = x * kc[a]
                        acc[m] = t if acc[m] is None else (acc[m] - t if c == 2 else acc[m] + t)
                        cnt += 2
                    if cnt >= cfg["G"] and not (c == 2 and i == iis[-1]):
                        yield cnt, [acc[m] for m in ms if acc[m] is not None]
                        cnt = 0
                for m in ms:
                    res[m, c] = acc[m]
            outs = []
            for m in ms:
                re, im = res[m, 2], res[m, 1]
                if not (last[m] and (m + 1 == NP or (m + 1 in ms and last[m + 1]))):
                    PS[m, R, L] = re
                    PS[m, R2, L] = im
                if last[m]:
                    if m > 0:
                        if m - 1 in ms:
                            assert last[m - 1]
                            pr, pi = res[m - 1, 2], res[m - 1, 1]
                        else:
                            pr, pi = PS[m - 1, R, L], PS[m - 1, R2, L]
                        re, im = (re - pi, im + pr) if qt in (0, 3) else (re + pi, im - pr)
                    Y[m, qt] = (re, im)
                outs += [re, im]
            yield cnt + 2 * len(outs), outs
            cnt = 0
        for m in ms:
            if not last[m]:
                continue
            (r0, i0), (r1, i1), (r2, i2), (r3, i3) = (Y[m, qt] for qt in range(4))
            ur0, ui0, vr0, vi0 = r0 + r2, i0 - i2, r0 - r2, i0 + i2
            ur1, ui1, vr1, vi1 = r1 + r3, i1 - i3, r1 - r3, i1 + i3
            ws = (ur0 + ur1, ui0 - ui1, vr0 - vi1, vi0 - vr1, ur0 - ur1, ui0 + ui1, vr0 + vi1, vi0 + vr1)
            for j, w in enumerate(ws):
                YS[m, 64 * j + 8 * g8:64 * j + 8 * g8 + 8, L] = w
            ymark[m, l] = ymark.get((m, l), 0) + 1
            yield 24, list(ws)

    def push_mac(ms, lim=NP):
        for idx in range(8 * NL):
            l, g = idx // 8, idx % 8
            terms, first, last = {}, {}, {}
            for m in ms:
                done = tdone.setdefault((m, idx), set())
                t = [i for i in range(m + 1) if i <= lim and m - i <= lim and i not in done]
                if not t:
                    continue
                for i in t:
                    assert ("x", i, l) in ready and ("k", m - i, l) in ready, (m, i)
                terms[m], first[m] = t, not done
                done.update(t)
                last[m] = len(done) == m + 1
                if last[m] and m > 0 and m - 1 not in ms:
                    assert len(tdone[m - 1, idx]) == m
            if terms:
                Q["mac"].append((min(ms), mac_gen(terms, first, last, g, l)))
        q = Q["mac"]
        head = q[:1] if q and st["cur"] is q[0] else []
        q[:] = head + sorted(q[len(head):], key=lambda e: e[0])

    def ln(x, scale=1.0):
        m = jnp.mean(x, axis=-1, keepdims=True)
        xc = x - m
        ss = jnp.sum(xc * xc, axis=-1, keepdims=True)
        r = jnp.exp(math.log(scale * math.sqrt(D)) - 0.5 * jnp.log(ss + D * EPS))
        return xc * r

    def lq_job(r0):
        xn = ln(qb[r0:r0 + 8, :].astype(f32))
        XN[r0:r0 + 8, :] = xn
        return [xn[:, LT(l)] for l in range(NL)]

    def push_lq(*ps):
        for p in ps:
            for g in range(32):
                Q["lq"].append([0, 34, functools.partial(lq_job, p * SB + 8 * g), p])

    def stage_c(p, ls):
        while any(ymark.get((p, l), 0) < 8 for l in ls):
            finish_mac()
        gm = pltpu.bitcast(gu[...], bf16)
        for l in ls:
            for c in range(4):
                YT[l, pl.ds(p * SB + c, 64, stride=4), :] = jnp.dot(
                    gm[64 * c:64 * c + 64], YS[p, 128 * c:128 * c + 128, LT(l)].astype(bf16),
                    preferred_element_type=f32)
        if ls[-1] != NL - 1:
            return

        def job(r0):
            force("lq", p)
            x = qb[r0:r0 + 8, :].astype(f32)
            h = x + XN[r0:r0 + 8, :] * jnp.concatenate([YT[l, r0:r0 + 8, :] for l in range(NL)], axis=1)
            HR[r0:r0 + 8, :] = h
            hn = ln(h, BETA)
            HN[r0:r0 + 8, :] = hn
            return [hn[:, LT(l)] for l in range(NL)]

        for g in range(32):
            Q["c"].append([cfg["c_delay"] if g == 0 else 0, 42, functools.partial(job, p * SB + 8 * g), p])

    def retile_w1(c0, c1):
        lo, hi = c0 * 128, min(c1 * 128, F)
        w1u[lo // 2:hi // 2, :] = pltpu.bitcast(w1t[lo:hi, :], u32)

    def retile_w2():
        w2u[...] = pltpu.bitcast(w2[...], u32)

    hs, os_ = {}, {}

    def stage_f1(b, nb, c0, c1, save):
        r0 = b * B
        force("c", b // 2)
        hn = cached(("hn", b), lambda: HN[r0:r0 + nb * B, :].astype(bf16))
        b1 = cached("b1", lambda: BETA * b1b[...].astype(f32)[None, :])
        out = {} if save else hs.setdefault(b, {})
        for c in range(c0, c1):
            lo, hi = c * 128, min((c + 1) * 128, F)
            w = pltpu.bitcast(w1u[lo // 2:hi // 2, :], bf16)
            init = linked_init(jnp.broadcast_to(b1[:, lo:hi], (nb * B, hi - lo)), cfg["cap1"] * 8)
            t = lax.dot_general(hn, w, NT, preferred_element_type=f32) + init
            out[c] = t + t * jnp.tanh(t * (KAPPA + t * t))
            if save:
                H1[r0:r0 + nb * B, lo:hi] = out[c]

    def stage_f2(b, nb, l0, l1):
        r0 = b * B
        if b in hs:
            if isinstance(hs[b], dict):
                hs[b] = tuple(jnp.concatenate([hs[b][c] for c in range(k0 // 128, (k1 + 127) // 128)],
                                              axis=1).astype(bf16) for k0, k1 in KG)
        else:
            hs[b] = tuple(H1[r0:r0 + nb * B, k0:k1].astype(bf16) for k0, k1 in KG)
        b2 = cached("b2", lambda: (1.0 / GAMMA) * b2b[...].astype(f32)[None, :])
        out = os_.setdefault(b, [])
        for l in range(l0, l1):
            o = jnp.broadcast_to(b2[:, LT(l)], (nb * B, 128))
            for (k0, k1), hk in zip(KG, hs[b]):
                o = jnp.dot(hk, pltpu.bitcast(w2u[k0 // 2:k1 // 2, LT(l)], bf16), preferred_element_type=f32
                            ) + linked_init(o, cfg["cap2"] * 8 * (k1 - k0) / 512)
            out.append(o)
        if l1 == NL:
            o = jnp.concatenate(os_.pop(b), axis=1)
            hs.pop(b)
            ob[r0:r0 + nb * B, :] = (HR[r0:r0 + nb * B, :] + GAMMA * o).astype(bf16)
            out_copy(b, nb).start()

    ops = dict(hold=lambda v: st.update(hold=v), set=lambda k, v: cfg.update({k: v}), tables=tables,
               kv=push_kv, kt=push_kt, lq=push_lq, x=stage_x, k=stage_k, mac=push_mac, c=stage_c,
               f1=stage_f1, f2=stage_f2, rw1=retile_w1, rw2=retile_w2)

    nreg = len(plan["prog"])
    for ridx, region in enumerate(plan["prog"]):
        @pl.when(pid == ridx)
        def _(region=region, ridx=ridx):
            if ridx > 0:
                st["never"] = lax.broadcasted_iota(jnp.int32, (8, 128), 0) < zs[0]
            st["cache"] = {}
            for step in region:
                if step[0] == "wait":
                    for c in groups[step[1]]:
                        c.wait()
                else:
                    ops[step[0]](*step[1:])
            if Q["mac"] and st["cur"] is Q["mac"][0]:
                finish_mac()
            for name in ("c", "kt", "kv", "lq"):
                while Q[name]:
                    Q[name].pop(0)[2]()
            st["credit"] = 0.0
            assert not hs and not os_ and not kvv
            if ridx == nreg - 1:
                assert not Q["mac"]
                out_copy(0, NB).wait()


def _plan():
    cfg = dict(G=32, cap1=1.6, cap2=2.2, capx=1.6, mul=1.0, maxcredit=40, c_delay=24)
    n1 = 5
    dma = [("s0", ["sk", ("s", 0, 2)]), ("a0", [("kv", 0, 1)]), ("q0", [("q", 0, 1), "small"]),
           ("g1", [("kv", 1, 2)]), ("w1a", [("w1", 0, n1)]), ("w1b", [("q", 1, 2), ("w1", n1, 11)]),
           ("g2", [("skvq", 2, 3)]), ("w2", [("w2", 0, 11)]), ("g3", [("skv", 3, 4)]),
           ("g4", [("q", 3, 4), ("skv", 4, 8)]), ("q4", [("q", 4, 8)])]
    A, Z = (0, 1), (2, 3)
    W = lambda n: [("wait", n)]
    kv = lambda *ps: [("kv", *ps)]
    kt = lambda *ps: [("kt", *ps)]
    lq = lambda *ps: [("lq", *ps)]
    K = lambda p, ls: [("k", p, ls)]
    X = lambda p, ls: [("x", p, ls)]
    C = lambda p: [("c", p, A), ("c", p, Z)]
    M = lambda m, lim=NP: [("mac", [m], lim)]
    F1 = lambda p, c0, c1: [("f1", 2 * p, 2, c0, c1, False)]
    S1 = lambda p, c0, c1: [("f1", 2 * p, 2, c0, c1, True)]
    F2 = lambda p, l0, l1: [("f2", 2 * p, 2, l0, l1)]
    FC = lambda p: lq(p + 1) + F1(p, 0, 11) + F2(p, 0, 1) + C(p + 1) + F2(p, 1, 4)
    prog = [
        [("tables",)] + W("s0") + kt(0, 1) + K(0, A) + K(0, Z),
        W("a0") + [("hold", True), ("set", "cap1", 2.2), ("set", "capx", 1.8)]
        + kv(0) + K(1, A) + X(0, A) + X(0, Z) + M(0) + K(1, Z) + C(0)
        + W("q0") + W("g1") + [("hold", False)] + lq(0) + kv(1) + X(1, A) + X(1, Z),
        W("w1a") + [("rw1", 0, n1), ("hold", True)] + M(1) + S1(0, 0, n1 - 1) + [("c", 1, A)]
        + S1(0, n1 - 1, n1) + [("c", 1, Z)]
        + W("w1b") + [("rw1", n1, 11)] + lq(1) + S1(0, n1, n1 + 2) + [("hold", False)] + S1(0, n1 + 2, 11),
        W("g2") + [("set", "cap1", cfg["cap1"]), ("set", "capx", cfg["capx"])] + kt(2) + kv(2) + lq(2) + M(2, 1)
        + S1(1, 0, 2) + K(2, A) + S1(1, 2, 4) + K(2, Z) + S1(1, 4, 6) + X(2, A) + S1(1, 6, 8) + X(2, Z)
        + S1(1, 8, 11),
        W("w2") + W("g3") + [("rw2",)] + M(2) + M(3, 2) + M(4, 2) + F2(0, 0, 3) + C(2)
        + kt(3) + kv(3) + F2(0, 3, 4) + F2(1, 0, 1) + K(3, A) + K(3, Z) + F2(1, 1, 2) + X(3, A) + F2(1, 2, 3)
        + X(3, Z) + F2(1, 3, 4),
        W("g4") + kt(4) + lq(3) + M(3) + M(4, 3) + M(5, 3) + F1(2, 0, 3)
        + K(4, A) + kt(5) + F1(2, 3, 4) + K(4, Z) + F1(2, 4, 5) + K(5, A) + kt(6) + F1(2, 5, 6) + K(5, Z)
        + F1(2, 6, 7) + K(6, A) + kt(7) + F1(2, 7, 8) + K(6, Z) + kv(4, 5, 6, 7) + F1(2, 8, 9) + K(7, A)
        + F1(2, 9, 10) + K(7, Z) + F1(2, 10, 11) + C(3) + F2(2, 0, 1) + X(4, A) + F2(2, 1, 2) + X(4, Z) + X(5, A)
        + F2(2, 2, 3) + X(5, Z) + F2(2, 3, 4) + X(6, A) + S1(3, 0, 1) + X(6, Z) + S1(3, 1, 2) + X(7, A)
        + S1(3, 2, 3) + X(7, Z),
        W("q4") + [("set", "mul", 0.9)] + lq(4) + M(4) + M(5) + M(6) + M(7)
        + S1(3, 3, 11) + F2(3, 0, 1) + C(4) + F2(3, 1, 4) + FC(4) + FC(5) + FC(6)
        + [("f1", 14, 1, 0, 11, False), ("f1", 15, 1, 0, 11, False), ("f2", 14, 1, 0, 4), ("f2", 15, 1, 0, 4)],
    ]
    return dict(dma=dma, prog=prog, cfg=cfg)


@jax.jit
def pallas_sequential_preLN__ssm_conv_h3__dense_activation_gelu__prompt_kernel(
    A_q: jax.Array,
    A_k: jax.Array,
    A_v: jax.Array,
    A_shift_k: jax.Array,
    A_ssm_k: jax.Array,
    A_ssm_D: jax.Array,
    B_x: jax.Array,
    B_w1: jax.Array,
    B_b1: jax.Array,
    B_w2: jax.Array,
    B_b2: jax.Array,
):
    plan = _plan()
    ANY = pl.BlockSpec(memory_space=pl.ANY)
    V = pltpu.VMEM
    scratch = [
        V((S, D), bf16), V((S, D), bf16), V((S, D), bf16), V((D, S), bf16),
        V((F, D), bf16), V((F, D), bf16),
        V((4, D), bf16), V((D,), bf16), V((F,), bf16), V((D,), bf16),
        V((NL, S + 16, 128), f32), V((S, D), bf16),
        V((F // 2, D), u32), V((F // 2, D), u32),
        V((128, 128), u32), V((128, 128), u32), V((128, 128), u32),
        V((NP, 3, SB, D), f32), V((NP, 3, SB, D), f32),
        V((NP, 2 * SB, D), f32), V((NP, 2 * SB, D), f32),
        V((S, D), f32), V((S, D), f32),
        V((4 * SB, F), f32), V((NL, S + 8, 128), f32), V((NL, S + 8, 128), f32),
        V((S, D), f32),
        pltpu.SMEM((1,), jnp.int32),
        pltpu.SemaphoreType.DMA((len(plan["dma"]),)), pltpu.SemaphoreType.DMA((1,)),
    ]
    out = pl.pallas_call(
        functools.partial(_kernel, plan=plan),
        grid=(len(plan["prog"]),),
        in_specs=[ANY] * 10,
        out_specs=ANY,
        out_shape=jax.ShapeDtypeStruct((S, D), bf16),
        scratch_shapes=scratch,
        compiler_params=pltpu.CompilerParams(
            dimension_semantics=("arbitrary",), vmem_limit_bytes=120 * 1024 * 1024,
            disable_semaphore_checks=True, disable_bounds_checks=True),
    )(A_q.reshape(S, D), A_k.reshape(S, D), A_v.reshape(S, D), A_shift_k.T, A_ssm_k, A_ssm_D,
      B_w1.T, B_b1, B_w2, B_b2)
    return out.reshape(1, S, D)
```

```python
import functools
import math

import jax
import jax.numpy as jnp
from jax import lax
import jax.experimental.pallas as pl
import jax.experimental.pallas.tpu as pltpu

S, D, F = 2048, 512, 1376
B = 128
NB = S // B
SB = 256
NP = S // SB
NL = D // 128
NF = (F + 127) // 128
EPS = 1e-5
f32, bf16, u32 = jnp.float32, jnp.bfloat16, jnp.uint32
NT = (((1,), (1,)), ((), ()))
C0 = math.sqrt(2.0 / math.pi)
C1 = C0 * 0.044715
KG = ((0, 512), (512, 1024), (1024, F))
BETA = C1 ** (1.0 / 3.0)
KAPPA = C0 / BETA
GAMMA = 0.5 / BETA


def _kernel(q_hbm, k_hbm, v_hbm, sk_hbm, ssm_hbm, sd_hbm, w1t_hbm, b1_hbm, w2_hbm, b2_hbm,
            o_hbm,
            qb, kb, vb, ssm, w1t, w2, skb, sdb, b1b, b2b, kf, ob,
            w1u, w2u, fe, fo, gu, XS, KS, PS, YS, HR, HN, H1, YT, KT, XN,
            zs, isem, osem, *, plan):
    cfg = dict(plan["cfg"])
    pid = pl.program_id(0)

    groups = {}
    for gi, (name, spec) in enumerate(plan["dma"]):
        cp = lambda src, dst: pltpu.make_async_copy(src, dst, isem.at[gi])
        cs = []
        for item in spec:
            if item == "sk":
                cs += [cp(sk_hbm, skb), cp(sd_hbm, sdb)]
            elif item == "small":
                cs += [cp(b1_hbm, b1b), cp(b2_hbm, b2b)]
            elif item[0] in ("w1", "w2"):
                src, dst = (w1t_hbm, w1t) if item[0] == "w1" else (w2_hbm, w2)
                r = pl.ds(item[1] * 128, min(item[2] * 128, F) - item[1] * 128)
                cs += [cp(src.at[r], dst.at[r])]
            else:
                r = pl.ds(item[1] * SB, (item[2] - item[1]) * SB)
                for ch in item[0]:
                    if ch == "s":
                        cs.append(cp(ssm_hbm.at[:, r], ssm.at[:, r]))
                    else:
                        src, dst = dict(k=(k_hbm, kb), v=(v_hbm, vb), q=(q_hbm, qb))[ch]
                        cs.append(cp(src.at[r], dst.at[r]))
        groups[name] = cs

    def out_copy(b, nb):
        r = pl.ds(b * B, nb * B)
        return pltpu.make_async_copy(ob.at[r], o_hbm.at[r], osem.at[0])

    Q = dict(c=[], kt=[], kv=[], lq=[], mac=[])
    st = dict(credit=0.0, never=None, cache={}, hold=False, cur=None)

    def cached(key, fn):
        if key not in st["cache"]:
            st["cache"][key] = fn()
        return st["cache"][key]

    def LT(l):
        return slice(l * 128, (l + 1) * 128)

    def tables():
        for cs in groups.values():
            for c in cs:
                c.start()
        zs[0] = 0

        def cosn(n, scale):
            n = jnp.abs((n & 1023) - 512)
            x = (n - 256).astype(f32) * (2.0 * math.pi / 1024)
            x2 = x * x
            p = -1.0 / 39916800.0
            for cf in (1.0 / 362880.0, -1.0 / 5040.0, 1.0 / 120.0, -1.0 / 6.0, 1.0):
                p = p * x2 + cf
            return p * (x * scale)

        r = lax.broadcasted_iota(jnp.int32, (256, 128), 0)
        c = lax.broadcasted_iota(jnp.int32, (256, 128), 1)
        slot_ = ((r >> 5) << 4) + (r & 15)
        odd = jnp.where(slot_ < 64, 4 * slot_ + 1, 511 - 4 * slot_)
        ne = odd * (2 * c) + ((r & 16) << 4)
        fe[...] = pltpu.bitcast(cosn(ne, 1.0).astype(bf16), u32)
        fo[...] = pltpu.bitcast(cosn(ne + odd, 1.0).astype(bf16), u32)
        j = 4 * (r & 63) + (r >> 6)
        gu[...] = pltpu.bitcast(cosn((4 * (c & 63) + 1) * j + ((c & 64) << 2), 1.0 / 256).astype(bf16), u32)
        for l in range(NL):
            kf[l, 0:8, :] = jnp.zeros((8, 128), f32)

    def take(cap):
        if st["never"] is None:
            return None
        st["credit"] = min(st["credit"] + cap * cfg["mul"], cfg["maxcredit"])
        deps = []
        for name in ("c", "kt", "kv", "lq"):
            q = Q[name]
            if name == "c" and st["hold"]:
                continue
            if q and q[0][0] > 0:
                q[0][0] -= 1
                continue
            while q and q[0][0] == 0 and st["credit"] > 0:
                j = q.pop(0)
                st["credit"] -= j[1]
                deps += j[2]()
        q = Q["mac"]
        while q and st["credit"] > 0:
            st["cur"] = q[0]
            nxt = next(q[0][1], None)
            if nxt is None:
                q.pop(0)
                continue
            st["credit"] -= nxt[0]
            deps += nxt[1]
        return functools.reduce(lambda x, y: x + y, deps) if deps else None

    def tie(piece, d):
        w = piece.shape[1]
        if w == 128:
            return lax.select(st["never"], d, piece)
        return lax.select(cached(("never", w), lambda: st["never"][:, :w]), d[:, :w], piece)

    def linked_init(init, cap):
        parts, start = [], 0
        for r in range(0, init.shape[0], 8):
            d = take(cap)
            if d is not None:
                if start < r:
                    parts.append(init[start:r])
                parts.append(tie(init[r:r + 8], d))
                start = r + 8
        if not parts:
            return init
        if start < init.shape[0]:
            parts.append(init[start:])
        return jnp.concatenate(parts, axis=0)

    def force(name, tag):
        while any(j[3] == tag for j in Q[name]):
            Q[name].pop(0)[2]()

    def finish_mac():
        for _ in Q["mac"].pop(0)[1]:
            pass

    kvv = {}

    def ku_job(r0):
        kall = kb[r0:r0 + 16, :].astype(f32)
        for l in range(NL):
            kf[l, 8 + r0:24 + r0, :] = kall[:, LT(l)]
        return [kall[8:16, LT(NL - 1)]]

    def kv_job(p, g, ls):
        r0 = p * SB + 16 * g
        sk = cached("sk", lambda: skb[...].astype(f32))
        outs = []
        for l in ls:
            vw = pltpu.bitcast(vb[r0:r0 + 16, LT(l)], u32)
            ve = pltpu.bitcast(vw << 16, f32)
            vo = pltpu.bitcast(vw & jnp.uint32(0xFFFF0000), f32)
            a = {o: kf[l, pl.ds(8 + r0 + o, 8, stride=2), :] for o in range(-3, 2)}
            w = [sk[t:t + 1, LT(l)] for t in range(4)]
            e = (a[0] * w[0] + a[-1] * w[1] + a[-2] * w[2] + a[-3] * w[3]) * ve
            o = (a[1] * w[0] + a[0] * w[1] + a[-1] * w[2] + a[-2] * w[3]) * vo
            kvv.setdefault((p, l), []).append((e, o))
            outs += [e, o]
        return outs

    def push_kv(*ps):
        for p in ps:
            for g in range(16):
                Q["kv"].append([0, 20, functools.partial(ku_job, p * SB + 16 * g), p])
        for p in ps:
            for g in range(16):
                for ls in ((0, 1), (2, 3)):
                    Q["kv"].append([0, 56, functools.partial(kv_job, p, g, ls), p])

    def kt_job(t0, l):
        t = jnp.transpose(ssm[LT(l), t0:t0 + 128].astype(f32))
        KT[l, t0:t0 + 128, :] = t
        return [t[120:128]]

    def push_kt(*ps):
        for p in ps:
            for l in range(NL):
                for h in range(2):
                    Q["kt"].append([0, 60, functools.partial(kt_job, p * SB + h * 128, l), p])

    ready = set()

    def fwd(p, ls, src, dst, is_k):
        fem, fom = pltpu.bitcast(fe[...], bf16), pltpu.bitcast(fo[...], bf16)
        res = {}
        for l in ls:
            ze, zo = src(l)
            res[l] = (jnp.dot(fem, ze.astype(bf16), preferred_element_type=f32),
                      jnp.dot(fom, zo.astype(bf16), preferred_element_type=f32))
        L = slice(128 * ls[0], 128 * ls[0] + 256)
        e = jnp.concatenate([res[l][0] for l in ls], axis=1)
        o = jnp.concatenate([res[l][1] for l in ls], axis=1)
        for g in range(16):
            r0 = (g // 2) * 32 + (g % 2) * 8
            er, ei, orr, oi = e[r0:r0 + 8], e[r0 + 16:r0 + 24], o[r0:r0 + 8], o[r0 + 16:r0 + 24]
            if is_k and p == 0:
                er = er + cached("sd", lambda: sdb[...].astype(f32)[None, :])[:, L]
            ds = [take(cfg["capx"] * 8) for _ in range(2)]
            if any(d is not None for d in ds):
                er = jnp.concatenate([er[:, LT(j)] if d is None else tie(er[:, LT(j)], d)
                                      for j, d in enumerate(ds)], axis=1)
            for rr, a, b in ((8 * g, er + orr, ei + oi), (128 + 8 * g, er - orr, oi - ei)):
                comps = (a, b - a, a + b) if is_k else (a + b, a, b)
                for ci, val in enumerate(comps):
                    dst[p, ci, rr:rr + 8, L] = val
        for l in ls:
            ready.add(("k" if is_k else "x", p, l))

    def stage_x(p, ls):
        force("kv", p)

        def src(l):
            eo = kvv.pop((p, l))
            return (jnp.concatenate([x[0] for x in eo], axis=0), jnp.concatenate([x[1] for x in eo], axis=0))

        fwd(p, ls, src, XS, False)

    def stage_k(p, ls):
        force("kt", p)
        fwd(p, ls, lambda l: (KT[l, pl.ds(p * SB, 128, stride=2), :], KT[l, pl.ds(p * SB + 1, 128, stride=2), :]),
            KS, True)

    ymark = {}
    tdone = {}

    def mac_gen(terms, first, last, g8, l):
        L = LT(l)
        ms = sorted(terms)
        iis = sorted(set(i for m in ms for i in terms[m]))
        Y = {}
        cnt = 0
        for qt in range(4):
            g = 8 * qt + g8
            R = slice(8 * g, 8 * g + 8)
            R2 = slice(SB + 8 * g, SB + 8 * g + 8)
            res = {}
            for c in range(3):
                kc = {}
                acc = {}
                for m in ms:
                    if c == 0:
                        acc[m] = None
                    elif first[m]:
                        acc[m] = res[m, 0]
                    else:
                        acc[m] = res[m, 0] + PS[m, R2 if c == 1 else R, L]
                        cnt += 1
                for i in iis:
                    x = XS[i, c, R, L]
                    for m in ms:
                        if i not in terms[m]:
                            continue
                        a = m - i
                        if a not in kc:
                            kc[a] = KS[a, c, R, L]
                        t = x * kc[a]
                        acc[m] = t if acc[m] is None else (acc[m] - t if c == 2 else acc[m] + t)
                        cnt += 2
                    if cnt >= cfg["G"] and not (c == 2 and i == iis[-1]):
                        yield cnt, [acc[m] for m in ms if acc[m] is not None]
                        cnt = 0
                for m in ms:
                    res[m, c] = acc[m]
            outs = []
            for m in ms:
                re, im = res[m, 2], res[m, 1]
                if not (last[m] and (m + 1 == NP or (m + 1 in ms and last[m + 1]))):
                    PS[m, R, L] = re
                    PS[m, R2, L] = im
                if last[m]:
                    if m > 0:
                        if m - 1 in ms:
                            assert last[m - 1]
                            pr, pi = res[m - 1, 2], res[m - 1, 1]
                        else:
                            pr, pi = PS[m - 1, R, L], PS[m - 1, R2, L]
                        re, im = (re - pi, im + pr) if qt in (0, 3) else (re + pi, im - pr)
                    Y[m, qt] = (re, im)
                outs += [re, im]
            yield cnt + 2 * len(outs), outs
            cnt = 0
        for m in ms:
            if not last[m]:
                continue
            (r0, i0), (r1, i1), (r2, i2), (r3, i3) = (Y[m, qt] for qt in range(4))
            ur0, ui0, vr0, vi0 = r0 + r2, i0 - i2, r0 - r2, i0 + i2
            ur1, ui1, vr1, vi1 = r1 + r3, i1 - i3, r1 - r3, i1 + i3
            ws = (ur0 + ur1, ui0 - ui1, vr0 - vi1, vi0 - vr1, ur0 - ur1, ui0 + ui1, vr0 + vi1, vi0 + vr1)
            for j, w in enumerate(ws):
                YS[m, 64 * j + 8 * g8:64 * j + 8 * g8 + 8, L] = w
            ymark[m, l] = ymark.get((m, l), 0) + 1
            yield 24, list(ws)

    def push_mac(ms, lim=NP):
        for idx in range(8 * NL):
            l, g = idx // 8, idx % 8
            terms, first, last = {}, {}, {}
            for m in ms:
                done = tdone.setdefault((m, idx), set())
                t = [i for i in range(m + 1) if i <= lim and m - i <= lim and i not in done]
                if not t:
                    continue
                for i in t:
                    assert ("x", i, l) in ready and ("k", m - i, l) in ready, (m, i)
                terms[m], first[m] = t, not done
                done.update(t)
                last[m] = len(done) == m + 1
                if last[m] and m > 0 and m - 1 not in ms:
                    assert len(tdone[m - 1, idx]) == m
            if terms:
                Q["mac"].append((min(ms), mac_gen(terms, first, last, g, l)))
        q = Q["mac"]
        head = q[:1] if q and st["cur"] is q[0] else []
        q[:] = head + sorted(q[len(head):], key=lambda e: e[0])

    def ln(x, scale=1.0):
        m = jnp.mean(x, axis=-1, keepdims=True)
        xc = x - m
        ss = jnp.sum(xc * xc, axis=-1, keepdims=True)
        r = jnp.exp(math.log(scale * math.sqrt(D)) - 0.5 * jnp.log(ss + D * EPS))
        return xc * r

    def lq_job(r0):
        xn = ln(qb[r0:r0 + 8, :].astype(f32))
        XN[r0:r0 + 8, :] = xn
        return [xn[:, LT(l)] for l in range(NL)]

    def push_lq(*ps):
        for p in ps:
            for g in range(32):
                Q["lq"].append([0, 34, functools.partial(lq_job, p * SB + 8 * g), p])

    def stage_c(p, ls):
        while any(ymark.get((p, l), 0) < 8 for l in ls):
            finish_mac()
        gm = pltpu.bitcast(gu[...], bf16)
        for l in ls:
            for c in range(4):
                YT[l, pl.ds(p * SB + c, 64, stride=4), :] = jnp.dot(
                    gm[64 * c:64 * c + 64], YS[p, 128 * c:128 * c + 128, LT(l)].astype(bf16),
                    preferred_element_type=f32)
        if ls[-1] != NL - 1:
            return

        def job(r0):
            force("lq", p)
            x = qb[r0:r0 + 8, :].astype(f32)
            h = x + XN[r0:r0 + 8, :] * jnp.concatenate([YT[l, r0:r0 + 8, :] for l in range(NL)], axis=1)
            HR[r0:r0 + 8, :] = h
            hn = ln(h, BETA)
            HN[r0:r0 + 8, :] = hn
            return [hn[:, LT(l)] for l in range(NL)]

        for g in range(32):
            Q["c"].append([cfg["c_delay"] if g == 0 else 0, 42, functools.partial(job, p * SB + 8 * g), p])

    def retile_w1(c0, c1):
        lo, hi = c0 * 128, min(c1 * 128, F)
        w1u[lo // 2:hi // 2, :] = pltpu.bitcast(w1t[lo:hi, :], u32)

    def retile_w2():
        w2u[...] = pltpu.bitcast(w2[...], u32)

    hs, os_ = {}, {}

    def stage_f1(b, nb, c0, c1, save):
        r0 = b * B
        force("c", b // 2)
        hn = cached(("hn", b), lambda: HN[r0:r0 + nb * B, :].astype(bf16))
        b1 = cached("b1", lambda: BETA * b1b[...].astype(f32)[None, :])
        out = {} if save else hs.setdefault(b, {})
        gelu2 = lambda t: t + t * jnp.tanh(t * (KAPPA + t * t))
        for c in range(c0, c1):
            if b >= 2:
                c = c if c < 8 else (NF - 1 if c == 8 else c - 1)
            lo, hi = c * 128, min((c + 1) * 128, F)
            n = hi - lo
            w = pltpu.bitcast(w1u[lo // 2:hi // 2, :], bf16)
            if n < 128 and b >= 2:
                bcol = cached("b1col", lambda: jnp.transpose(jnp.broadcast_to(
                    jnp.concatenate([b1[:, lo:hi], b1[:, :128 - n]], axis=1), (128, 128)))[:n])
                t = lax.dot_general(w, hn, NT, preferred_element_type=f32)
                gs = [gelu2(t[:, LT(rb)] + linked_init(bcol, cfg["cap1"] * 8)) for rb in range(nb)]
                out[c] = jnp.concatenate(
                    [jnp.transpose(jnp.concatenate([g, g[:128 - n]], axis=0))[:, :n] for g in gs], axis=0)
            else:
                init = linked_init(jnp.broadcast_to(b1[:, lo:hi], (nb * B, n)), cfg["cap1"] * 8)
                out[c] = gelu2(lax.dot_general(hn, w, NT, preferred_element_type=f32) + init)
            if save:
                H1[r0:r0 + nb * B, lo:hi] = out[c]

    def stage_f2(b, nb, l0, l1):
        r0 = b * B
        if b in hs:
            if isinstance(hs[b], dict):
                hs[b] = tuple(jnp.concatenate([hs[b][c] for c in range(k0 // 128, (k1 + 127) // 128)],
                                              axis=1).astype(bf16) for k0, k1 in KG)
        else:
            hs[b] = tuple(H1[r0:r0 + nb * B, k0:k1].astype(bf16) for k0, k1 in KG)
        b2 = cached("b2", lambda: (1.0 / GAMMA) * b2b[...].astype(f32)[None, :])
        out = os_.setdefault(b, [])
        for l in range(l0, l1):
            o = jnp.broadcast_to(b2[:, LT(l)], (nb * B, 128))
            for (k0, k1), hk in zip(KG, hs[b]):
                o = jnp.dot(hk, pltpu.bitcast(w2u[k0 // 2:k1 // 2, LT(l)], bf16), preferred_element_type=f32
                            ) + linked_init(o, cfg["cap2"] * 8 * (k1 - k0) / 512)
            out.append(o)
        if l1 == NL:
            o = jnp.concatenate(os_.pop(b), axis=1)
            hs.pop(b)
            ob[r0:r0 + nb * B, :] = (HR[r0:r0 + nb * B, :] + GAMMA * o).astype(bf16)
            out_copy(b, nb).start()

    ops = dict(hold=lambda v: st.update(hold=v), set=lambda k, v: cfg.update({k: v}), tables=tables,
               kv=push_kv, kt=push_kt, lq=push_lq, x=stage_x, k=stage_k, mac=push_mac, c=stage_c,
               f1=stage_f1, f2=stage_f2, rw1=retile_w1, rw2=retile_w2)

    nreg = len(plan["prog"])
    for ridx, region in enumerate(plan["prog"]):
        @pl.when(pid == ridx)
        def _(region=region, ridx=ridx):
            if ridx > 0:
                st["never"] = lax.broadcasted_iota(jnp.int32, (8, 128), 0) < zs[0]
            st["cache"] = {}
            for step in region:
                if step[0] == "wait":
                    for c in groups[step[1]]:
                        c.wait()
                else:
                    ops[step[0]](*step[1:])
            if Q["mac"] and st["cur"] is Q["mac"][0]:
                finish_mac()
            for name in ("c", "kt", "kv", "lq"):
                while Q[name]:
                    Q[name].pop(0)[2]()
            st["credit"] = 0.0
            assert not hs and not os_ and not kvv
            if ridx == nreg - 1:
                assert not Q["mac"]
                out_copy(0, NB).wait()


def _plan():
    cfg = dict(G=32, cap1=1.6, cap2=2.2, capx=1.6, mul=1.0, maxcredit=40, c_delay=24)
    n1 = 5
    dma = [("s0", ["sk", ("s", 0, 2)]), ("a0", [("kv", 0, 1)]), ("q0", [("q", 0, 1), "small"]),
           ("g1", [("kv", 1, 2)]), ("w1a", [("w1", 0, n1)]), ("w1b", [("q", 1, 2), ("w1", n1, 11)]),
           ("g2", [("skvq", 2, 3)]), ("w2", [("w2", 0, 11)]), ("g3", [("skv", 3, 4)]),
           ("g4", [("q", 3, 4), ("skv", 4, 8)]), ("q4", [("q", 4, 8)])]
    A, Z = (0, 1), (2, 3)
    W = lambda n: [("wait", n)]
    kv = lambda *ps: [("kv", *ps)]
    kt = lambda *ps: [("kt", *ps)]
    lq = lambda *ps: [("lq", *ps)]
    K = lambda p, ls: [("k", p, ls)]
    X = lambda p, ls: [("x", p, ls)]
    C = lambda p: [("c", p, A), ("c", p, Z)]
    M = lambda m, lim=NP: [("mac", [m], lim)]
    F1 = lambda p, c0, c1: [("f1", 2 * p, 2, c0, c1, False)]
    S1 = lambda p, c0, c1: [("f1", 2 * p, 2, c0, c1, True)]
    F2 = lambda p, l0, l1: [("f2", 2 * p, 2, l0, l1)]
    FC = lambda p: lq(p + 1) + F1(p, 0, 11) + F2(p, 0, 1) + C(p + 1) + F2(p, 1, 4)
    prog = [
        [("tables",)] + W("s0") + kt(0, 1) + K(0, A) + K(0, Z),
        W("a0") + [("hold", True), ("set", "cap1", 2.2), ("set", "capx", 1.8)]
        + kv(0) + K(1, A) + X(0, A) + X(0, Z) + M(0) + K(1, Z) + C(0)
        + W("q0") + W("g1") + [("hold", False)] + lq(0) + kv(1) + X(1, A) + X(1, Z),
        W("w1a") + [("rw1", 0, n1), ("hold", True)] + M(1) + S1(0, 0, n1 - 1) + [("c", 1, A)]
        + S1(0, n1 - 1, n1) + [("c", 1, Z)]
        + W("w1b") + [("rw1", n1, 11)] + lq(1) + S1(0, n1, n1 + 2) + [("hold", False)] + S1(0, n1 + 2, 11),
        W("g2") + [("set", "cap1", cfg["cap1"]), ("set", "capx", cfg["capx"])] + kt(2) + kv(2) + lq(2) + M(2, 1)
        + S1(1, 0, 2) + K(2, A) + S1(1, 2, 4) + K(2, Z) + S1(1, 4, 6) + X(2, A) + S1(1, 6, 8) + X(2, Z)
        + S1(1, 8, 11),
        W("w2") + W("g3") + [("rw2",)] + M(2) + M(3, 2) + M(4, 2) + F2(0, 0, 3) + C(2)
        + kt(3) + kv(3) + F2(0, 3, 4) + F2(1, 0, 1) + K(3, A) + K(3, Z) + F2(1, 1, 2) + X(3, A) + F2(1, 2, 3)
        + X(3, Z) + F2(1, 3, 4),
        W("g4") + kt(4) + lq(3) + M(3) + M(4, 3) + M(5, 3) + F1(2, 0, 3)
        + K(4, A) + kt(5) + F1(2, 3, 4) + K(4, Z) + F1(2, 4, 5) + K(5, A) + kt(6) + F1(2, 5, 6) + K(5, Z)
        + F1(2, 6, 7) + K(6, A) + kt(7) + F1(2, 7, 8) + K(6, Z) + kv(4, 5, 6, 7) + F1(2, 8, 9) + K(7, A)
        + F1(2, 9, 10) + K(7, Z) + F1(2, 10, 11) + C(3) + F2(2, 0, 1) + X(4, A) + F2(2, 1, 2) + X(4, Z) + X(5, A)
        + F2(2, 2, 3) + X(5, Z) + F2(2, 3, 4) + X(6, A) + S1(3, 0, 1) + X(6, Z) + S1(3, 1, 2) + X(7, A)
        + S1(3, 2, 3) + X(7, Z),
        W("q4") + [("set", "mul", 0.9)] + lq(4) + M(4) + M(5) + M(6) + M(7)
        + S1(3, 3, 11) + F2(3, 0, 1) + C(4) + F2(3, 1, 4) + FC(4) + FC(5) + FC(6)
        + [("f1", 14, 1, 0, 11, False), ("f1", 15, 1, 0, 11, False), ("f2", 14, 1, 0, 4), ("f2", 15, 1, 0, 4)],
    ]
    return dict(dma=dma, prog=prog, cfg=cfg)


@jax.jit
def pallas_sequential_preLN__ssm_conv_h3__dense_activation_gelu__prompt_kernel(
    A_q: jax.Array,
    A_k: jax.Array,
    A_v: jax.Array,
    A_shift_k: jax.Array,
    A_ssm_k: jax.Array,
    A_ssm_D: jax.Array,
    B_x: jax.Array,
    B_w1: jax.Array,
    B_b1: jax.Array,
    B_w2: jax.Array,
    B_b2: jax.Array,
):
    plan = _plan()
    ANY = pl.BlockSpec(memory_space=pl.ANY)
    V = pltpu.VMEM
    scratch = [
        V((S, D), bf16), V((S, D), bf16), V((S, D), bf16), V((D, S), bf16),
        V((F, D), bf16), V((F, D), bf16),
        V((4, D), bf16), V((D,), bf16), V((F,), bf16), V((D,), bf16),
        V((NL, S + 16, 128), f32), V((S, D), bf16),
        V((F // 2, D), u32), V((F // 2, D), u32),
        V((128, 128), u32), V((128, 128), u32), V((128, 128), u32),
        V((NP, 3, SB, D), f32), V((NP, 3, SB, D), f32),
        V((NP, 2 * SB, D), f32), V((NP, 2 * SB, D), f32),
        V((S, D), f32), V((S, D), f32),
        V((4 * SB, F), f32), V((NL, S + 8, 128), f32), V((NL, S + 8, 128), f32),
        V((S, D), f32),
        pltpu.SMEM((1,), jnp.int32),
        pltpu.SemaphoreType.DMA((len(plan["dma"]),)), pltpu.SemaphoreType.DMA((1,)),
    ]
    out = pl.pallas_call(
        functools.partial(_kernel, plan=plan),
        grid=(len(plan["prog"]),),
        in_specs=[ANY] * 10,
        out_specs=ANY,
        out_shape=jax.ShapeDtypeStruct((S, D), bf16),
        scratch_shapes=scratch,
        compiler_params=pltpu.CompilerParams(
            dimension_semantics=("arbitrary",), vmem_limit_bytes=120 * 1024 * 1024,
            disable_semaphore_checks=True, disable_bounds_checks=True),
    )(A_q.reshape(S, D), A_k.reshape(S, D), A_v.reshape(S, D), A_shift_k.T, A_ssm_k, A_ssm_D,
      B_w1.T, B_b1, B_w2, B_b2)
    return out.reshape(1, S, D)
```

```python
import functools
import math

import jax
import jax.numpy as jnp
from jax import lax
import jax.experimental.pallas as pl
import jax.experimental.pallas.tpu as pltpu

S, D, F = 2048, 512, 1376
B = 128
NB = S // B
SB = 256
NP = S // SB
NL = D // 128
NF = (F + 127) // 128
EPS = 1e-5
f32, bf16, u32 = jnp.float32, jnp.bfloat16, jnp.uint32
NT = (((1,), (1,)), ((), ()))
C0 = math.sqrt(2.0 / math.pi)
C1 = C0 * 0.044715
KG = ((0, 512), (512, 1024), (1024, F))
BETA = C1 ** (1.0 / 3.0)
KAPPA = C0 / BETA
GAMMA = 0.5 / BETA


def _kernel(q_hbm, k_hbm, v_hbm, sk_hbm, ssm_hbm, sd_hbm, w1t_hbm, b1_hbm, w2_hbm, b2_hbm,
            o_hbm,
            qb, kb, vb, ssm, w1t, w2, skb, sdb, b1b, b2b, kf, ob,
            w1u, w2u, fe, fo, gu, XS, KS, PS, YS, HR, HN, H1, YT, KT, XN,
            zs, isem, osem, *, plan):
    cfg = dict(plan["cfg"])
    pid = pl.program_id(0)

    groups = {}
    for gi, (name, spec) in enumerate(plan["dma"]):
        cp = lambda src, dst: pltpu.make_async_copy(src, dst, isem.at[gi])
        cs = []
        for item in spec:
            if item == "sk":
                cs += [cp(sk_hbm, skb), cp(sd_hbm, sdb)]
            elif item == "small":
                cs += [cp(b1_hbm, b1b), cp(b2_hbm, b2b)]
            elif item[0] in ("w1", "w2"):
                src, dst = (w1t_hbm, w1t) if item[0] == "w1" else (w2_hbm, w2)
                r = pl.ds(item[1] * 128, min(item[2] * 128, F) - item[1] * 128)
                cs += [cp(src.at[r], dst.at[r])]
            else:
                r = pl.ds(item[1] * SB, (item[2] - item[1]) * SB)
                for ch in item[0]:
                    if ch == "s":
                        cs.append(cp(ssm_hbm.at[:, r], ssm.at[:, r]))
                    else:
                        src, dst = dict(k=(k_hbm, kb), v=(v_hbm, vb), q=(q_hbm, qb))[ch]
                        cs.append(cp(src.at[r], dst.at[r]))
        groups[name] = cs

    def out_copy(b, nb):
        r = pl.ds(b * B, nb * B)
        return pltpu.make_async_copy(ob.at[r], o_hbm.at[r], osem.at[0])

    Q = dict(c=[], kt=[], kv=[], lq=[], mac=[])
    st = dict(credit=0.0, never=None, cache={}, hold=False, cur=None)

    def cached(key, fn):
        if key not in st["cache"]:
            st["cache"][key] = fn()
        return st["cache"][key]

    def LT(l):
        return slice(l * 128, (l + 1) * 128)

    def tables():
        for cs in groups.values():
            for c in cs:
                c.start()
        zs[0] = 0

        def cosn(n, scale):
            n = jnp.abs((n & 1023) - 512)
            x = (n - 256).astype(f32) * (2.0 * math.pi / 1024)
            x2 = x * x
            p = -1.0 / 39916800.0
            for cf in (1.0 / 362880.0, -1.0 / 5040.0, 1.0 / 120.0, -1.0 / 6.0, 1.0):
                p = p * x2 + cf
            return p * (x * scale)

        r = lax.broadcasted_iota(jnp.int32, (256, 128), 0)
        c = lax.broadcasted_iota(jnp.int32, (256, 128), 1)
        slot_ = ((r >> 5) << 4) + (r & 15)
        odd = jnp.where(slot_ < 64, 4 * slot_ + 1, 511 - 4 * slot_)
        ne = odd * (2 * c) + ((r & 16) << 4)
        fe[...] = pltpu.bitcast(cosn(ne, 1.0).astype(bf16), u32)
        fo[...] = pltpu.bitcast(cosn(ne + odd, 1.0).astype(bf16), u32)
        j = 4 * (r & 63) + (r >> 6)
        gu[...] = pltpu.bitcast(cosn((4 * (c & 63) + 1) * j + ((c & 64) << 2), 1.0 / 256).astype(bf16), u32)
        for l in range(NL):
            kf[l, 0:8, :] = jnp.zeros((8, 128), f32)

    def take(cap):
        if st["never"] is None:
            return None
        st["credit"] = min(st["credit"] + cap * cfg["mul"], cfg["maxcredit"])
        deps = []
        for name in ("c", "kt", "kv", "lq"):
            q = Q[name]
            if name == "c" and st["hold"]:
                continue
            if q and q[0][0] > 0:
                q[0][0] -= 1
                continue
            while q and q[0][0] == 0 and st["credit"] > 0:
                j = q.pop(0)
                st["credit"] -= j[1]
                deps += j[2]()
        q = Q["mac"]
        while q and st["credit"] > 0:
            st["cur"] = q[0]
            nxt = next(q[0][1], None)
            if nxt is None:
                q.pop(0)
                continue
            st["credit"] -= nxt[0]
            deps += nxt[1]
        return functools.reduce(lambda x, y: x + y, deps) if deps else None

    def tie(piece, d):
        w = piece.shape[1]
        if w == 128:
            return lax.select(st["never"], d, piece)
        return lax.select(cached(("never", w), lambda: st["never"][:, :w]), d[:, :w], piece)

    def linked_init(init, cap):
        parts, start = [], 0
        for r in range(0, init.shape[0], 8):
            d = take(cap)
            if d is not None:
                if start < r:
                    parts.append(init[start:r])
                parts.append(tie(init[r:r + 8], d))
                start = r + 8
        if not parts:
            return init
        if start < init.shape[0]:
            parts.append(init[start:])
        return jnp.concatenate(parts, axis=0)

    def force(name, tag):
        while any(j[3] == tag for j in Q[name]):
            Q[name].pop(0)[2]()

    def finish_mac():
        for _ in Q["mac"].pop(0)[1]:
            pass

    kvv = {}

    def ku_job(r0):
        kall = kb[r0:r0 + 16, :].astype(f32)
        for l in range(NL):
            kf[l, 8 + r0:24 + r0, :] = kall[:, LT(l)]
        return [kall[8:16, LT(NL - 1)]]

    def kv_job(p, g, ls):
        r0 = p * SB + 16 * g
        sk = cached("sk", lambda: skb[...].astype(f32))
        outs = []
        for l in ls:
            vw = pltpu.bitcast(vb[r0:r0 + 16, LT(l)], u32)
            ve = pltpu.bitcast(vw << 16, f32)
            vo = pltpu.bitcast(vw & jnp.uint32(0xFFFF0000), f32)
            a = {o: kf[l, pl.ds(8 + r0 + o, 8, stride=2), :] for o in range(-3, 2)}
            w = [sk[t:t + 1, LT(l)] for t in range(4)]
            e = (a[0] * w[0] + a[-1] * w[1] + a[-2] * w[2] + a[-3] * w[3]) * ve
            o = (a[1] * w[0] + a[0] * w[1] + a[-1] * w[2] + a[-2] * w[3]) * vo
            kvv.setdefault((p, l), []).append((e, o))
            outs += [e, o]
        return outs

    def push_kv(*ps):
        for p in ps:
            for g in range(16):
                Q["kv"].append([0, 20, functools.partial(ku_job, p * SB + 16 * g), p])
        for p in ps:
            for g in range(16):
                for ls in ((0, 1), (2, 3)):
                    Q["kv"].append([0, 56, functools.partial(kv_job, p, g, ls), p])

    def kt_job(t0, l):
        t = jnp.transpose(ssm[LT(l), t0:t0 + 128].astype(f32))
        KT[l, t0:t0 + 128, :] = t
        return [t[120:128]]

    def push_kt(*ps):
        for p in ps:
            for l in range(NL):
                for h in range(2):
                    Q["kt"].append([0, 60, functools.partial(kt_job, p * SB + h * 128, l), p])

    ready = set()

    def fwd(p, ls, src, dst, is_k):
        fem, fom = pltpu.bitcast(fe[...], bf16), pltpu.bitcast(fo[...], bf16)
        res = {}
        for l in ls:
            ze, zo = src(l)
            res[l] = (jnp.dot(fem, ze.astype(bf16), preferred_element_type=f32),
                      jnp.dot(fom, zo.astype(bf16), preferred_element_type=f32))
        L = slice(128 * ls[0], 128 * ls[0] + 256)
        e = jnp.concatenate([res[l][0] for l in ls], axis=1)
        o = jnp.concatenate([res[l][1] for l in ls], axis=1)
        for g in range(16):
            r0 = (g // 2) * 32 + (g % 2) * 8
            er, ei, orr, oi = e[r0:r0 + 8], e[r0 + 16:r0 + 24], o[r0:r0 + 8], o[r0 + 16:r0 + 24]
            if is_k and p == 0:
                er = er + cached("sd", lambda: sdb[...].astype(f32)[None, :])[:, L]
            ds = [take(cfg["capx"] * 8) for _ in range(2)]
            if any(d is not None for d in ds):
                er = jnp.concatenate([er[:, LT(j)] if d is None else tie(er[:, LT(j)], d)
                                      for j, d in enumerate(ds)], axis=1)
            for rr, a, b in ((8 * g, er + orr, ei + oi), (128 + 8 * g, er - orr, oi - ei)):
                comps = (a, b - a, a + b) if is_k else (a + b, a, b)
                for ci, val in enumerate(comps):
                    dst[p, ci, rr:rr + 8, L] = val
        for l in ls:
            ready.add(("k" if is_k else "x", p, l))

    def stage_x(p, ls):
        force("kv", p)

        def src(l):
            eo = kvv.pop((p, l))
            return (jnp.concatenate([x[0] for x in eo], axis=0), jnp.concatenate([x[1] for x in eo], axis=0))

        fwd(p, ls, src, XS, False)

    def stage_k(p, ls):
        force("kt", p)
        fwd(p, ls, lambda l: (KT[l, pl.ds(p * SB, 128, stride=2), :], KT[l, pl.ds(p * SB + 1, 128, stride=2), :]),
            KS, True)

    ymark = {}
    tdone = {}

    def mac_gen(terms, first, last, g8, l):
        L = LT(l)
        ms = sorted(terms)
        iis = sorted(set(i for m in ms for i in terms[m]))
        Y = {}
        cnt = 0
        for qt in range(4):
            g = 8 * qt + g8
            R = slice(8 * g, 8 * g + 8)
            R2 = slice(SB + 8 * g, SB + 8 * g + 8)
            res = {}
            for c in range(3):
                kc = {}
                acc = {}
                for m in ms:
                    if c == 0:
                        acc[m] = None
                    elif first[m]:
                        acc[m] = res[m, 0]
                    else:
                        acc[m] = res[m, 0] + PS[m, R2 if c == 1 else R, L]
                        cnt += 1
                for i in iis:
                    x = XS[i, c, R, L]
                    for m in ms:
                        if i not in terms[m]:
                            continue
                        a = m - i
                        if a not in kc:
                            kc[a] = KS[a, c, R, L]
                        t = x * kc[a]
                        acc[m] = t if acc[m] is None else (acc[m] - t if c == 2 else acc[m] + t)
                        cnt += 2
                    if cnt >= cfg["G"] and not (c == 2 and i == iis[-1]):
                        yield cnt, [acc[m] for m in ms if acc[m] is not None]
                        cnt = 0
                for m in ms:
                    res[m, c] = acc[m]
            outs = []
            for m in ms:
                re, im = res[m, 2], res[m, 1]
                if not (last[m] and (m + 1 == NP or (m + 1 in ms and last[m + 1]))):
                    PS[m, R, L] = re
                    PS[m, R2, L] = im
                if last[m]:
                    if m > 0:
                        if m - 1 in ms:
                            assert last[m - 1]
                            pr, pi = res[m - 1, 2], res[m - 1, 1]
                        else:
                            pr, pi = PS[m - 1, R, L], PS[m - 1, R2, L]
                        re, im = (re - pi, im + pr) if qt in (0, 3) else (re + pi, im - pr)
                    Y[m, qt] = (re, im)
                outs += [re, im]
            yield cnt + 2 * len(outs), outs
            cnt = 0
        for m in ms:
            if not last[m]:
                continue
            (r0, i0), (r1, i1), (r2, i2), (r3, i3) = (Y[m, qt] for qt in range(4))
            ur0, ui0, vr0, vi0 = r0 + r2, i0 - i2, r0 - r2, i0 + i2
            ur1, ui1, vr1, vi1 = r1 + r3, i1 - i3, r1 - r3, i1 + i3
            ws = (ur0 + ur1, ui0 - ui1, vr0 - vi1, vi0 - vr1, ur0 - ur1, ui0 + ui1, vr0 + vi1, vi0 + vr1)
            for j, w in enumerate(ws):
                YS[m, 64 * j + 8 * g8:64 * j + 8 * g8 + 8, L] = w
            ymark[m, l] = ymark.get((m, l), 0) + 1
            yield 24, list(ws)

    def push_mac(ms, lim=NP):
        for idx in range(8 * NL):
            l, g = idx // 8, idx % 8
            terms, first, last = {}, {}, {}
            for m in ms:
                done = tdone.setdefault((m, idx), set())
                t = [i for i in range(m + 1) if i <= lim and m - i <= lim and i not in done]
                if not t:
                    continue
                for i in t:
                    assert ("x", i, l) in ready and ("k", m - i, l) in ready, (m, i)
                terms[m], first[m] = t, not done
                done.update(t)
                last[m] = len(done) == m + 1
                if last[m] and m > 0 and m - 1 not in ms:
                    assert len(tdone[m - 1, idx]) == m
            if terms:
                Q["mac"].append((min(ms), mac_gen(terms, first, last, g, l)))
        q = Q["mac"]
        head = q[:1] if q and st["cur"] is q[0] else []
        q[:] = head + sorted(q[len(head):], key=lambda e: e[0])

    def ln(x, scale=1.0):
        m = jnp.mean(x, axis=-1, keepdims=True)
        xc = x - m
        ss = jnp.sum(xc * xc, axis=-1, keepdims=True)
        r = lax.rsqrt(ss * (1.0 / (D * scale * scale)) + EPS / (scale * scale))
        return xc * r

    def lq_job(r0):
        xn = ln(qb[r0:r0 + 8, :].astype(f32))
        XN[r0:r0 + 8, :] = xn
        return [xn[:, LT(l)] for l in range(NL)]

    def push_lq(*ps):
        for p in ps:
            for g in range(32):
                Q["lq"].append([0, 34, functools.partial(lq_job, p * SB + 8 * g), p])

    def stage_c(p, ls):
        while any(ymark.get((p, l), 0) < 8 for l in ls):
            finish_mac()
        gm = pltpu.bitcast(gu[...], bf16)
        for l in ls:
            for c in range(4):
                YT[l, pl.ds(p * SB + c, 64, stride=4), :] = jnp.dot(
                    gm[64 * c:64 * c + 64], YS[p, 128 * c:128 * c + 128, LT(l)].astype(bf16),
                    preferred_element_type=f32)
        if ls[-1] != NL - 1:
            return

        def job(r0):
            force("lq", p)
            x = qb[r0:r0 + 8, :].astype(f32)
            h = x + XN[r0:r0 + 8, :] * jnp.concatenate([YT[l, r0:r0 + 8, :] for l in range(NL)], axis=1)
            HR[r0:r0 + 8, :] = h
            hn = ln(h, BETA)
            HN[r0:r0 + 8, :] = hn
            return [hn[:, LT(l)] for l in range(NL)]

        for g in range(32):
            Q["c"].append([cfg["c_delay"] if g == 0 else 0, 42, functools.partial(job, p * SB + 8 * g), p])

    def retile_w1(c0, c1):
        lo, hi = c0 * 128, min(c1 * 128, F)
        w1u[lo // 2:hi // 2, :] = pltpu.bitcast(w1t[lo:hi, :], u32)

    def retile_w2():
        w2u[...] = pltpu.bitcast(w2[...], u32)

    hs, os_ = {}, {}

    def stage_f1(b, nb, c0, c1, save):
        r0 = b * B
        force("c", b // 2)
        hn = cached(("hn", b), lambda: HN[r0:r0 + nb * B, :].astype(bf16))
        b1 = cached("b1", lambda: BETA * b1b[...].astype(f32)[None, :])
        out = {} if save else hs.setdefault(b, {})
        gelu2 = lambda t: t + t * jnp.tanh(t * (KAPPA + t * t))
        for c in range(c0, c1):
            if b >= 2:
                c = c if c < 9 else 19 - c
            lo, hi = c * 128, min((c + 1) * 128, F)
            n = hi - lo
            w = pltpu.bitcast(w1u[lo // 2:hi // 2, :], bf16)
            if n < 128 and b >= 2:
                bcol = cached("b1col", lambda: jnp.transpose(jnp.broadcast_to(
                    jnp.concatenate([b1[:, lo:hi], b1[:, :128 - n]], axis=1), (128, 128)))[:n])
                t = lax.dot_general(w, hn, NT, preferred_element_type=f32)
                gs = [gelu2(t[:, LT(rb)] + linked_init(bcol, cfg["cap1"] * 8)) for rb in range(nb)]
                out[c] = jnp.concatenate(
                    [jnp.transpose(jnp.concatenate([g, g[:128 - n]], axis=0))[:, :n] for g in gs], axis=0)
            else:
                init = linked_init(jnp.broadcast_to(b1[:, lo:hi], (nb * B, n)), cfg["cap1"] * 8)
                out[c] = gelu2(lax.dot_general(hn, w, NT, preferred_element_type=f32) + init)
            if save:
                H1[r0:r0 + nb * B, lo:hi] = out[c]

    def stage_f2(b, nb, l0, l1):
        r0 = b * B
        if b in hs:
            if isinstance(hs[b], dict):
                hs[b] = tuple(jnp.concatenate([hs[b][c] for c in range(k0 // 128, (k1 + 127) // 128)],
                                              axis=1).astype(bf16) for k0, k1 in KG)
        else:
            hs[b] = tuple(H1[r0:r0 + nb * B, k0:k1].astype(bf16) for k0, k1 in KG)
        b2 = cached("b2", lambda: (1.0 / GAMMA) * b2b[...].astype(f32)[None, :])
        out = os_.setdefault(b, [])
        for l in range(l0, l1):
            o = jnp.broadcast_to(b2[:, LT(l)], (nb * B, 128))
            for (k0, k1), hk in zip(KG, hs[b]):
                o = jnp.dot(hk, pltpu.bitcast(w2u[k0 // 2:k1 // 2, LT(l)], bf16), preferred_element_type=f32
                            ) + linked_init(o, cfg["cap2"] * 8 * (k1 - k0) / 512)
            out.append(o)
        if l1 == NL:
            o = jnp.concatenate(os_.pop(b), axis=1)
            hs.pop(b)
            ob[r0:r0 + nb * B, :] = (HR[r0:r0 + nb * B, :] + GAMMA * o).astype(bf16)
            out_copy(b, nb).start()

    ops = dict(hold=lambda v: st.update(hold=v), set=lambda k, v: cfg.update({k: v}), tables=tables,
               kv=push_kv, kt=push_kt, lq=push_lq, x=stage_x, k=stage_k, mac=push_mac, c=stage_c,
               f1=stage_f1, f2=stage_f2, rw1=retile_w1, rw2=retile_w2)

    nreg = len(plan["prog"])
    for ridx, region in enumerate(plan["prog"]):
        @pl.when(pid == ridx)
        def _(region=region, ridx=ridx):
            if ridx > 0:
                st["never"] = lax.broadcasted_iota(jnp.int32, (8, 128), 0) < zs[0]
            st["cache"] = {}
            for step in region:
                if step[0] == "wait":
                    for c in groups[step[1]]:
                        c.wait()
                else:
                    ops[step[0]](*step[1:])
            if Q["mac"] and st["cur"] is Q["mac"][0]:
                finish_mac()
            for name in ("c", "kt", "kv", "lq"):
                while Q[name]:
                    Q[name].pop(0)[2]()
            st["credit"] = 0.0
            assert not hs and not os_ and not kvv
            if ridx == nreg - 1:
                assert not Q["mac"]
                out_copy(0, NB).wait()


def _plan():
    cfg = dict(G=32, cap1=1.7, cap2=2.1, capx=1.6, mul=1.0, maxcredit=40, c_delay=24)
    n1 = 5
    dma = [("s0", ["sk", ("s", 0, 2)]), ("a0", [("kv", 0, 1)]), ("q0", [("q", 0, 1), "small"]),
           ("g1", [("kv", 1, 2)]), ("w1a", [("w1", 0, n1)]), ("w1b", [("q", 1, 2), ("w1", n1, 11)]),
           ("g2", [("skvq", 2, 3)]), ("w2", [("w2", 0, 11)]), ("g3", [("skv", 3, 4)]),
           ("g4", [("q", 3, 4), ("skv", 4, 8)]), ("q4", [("q", 4, 8)])]
    A, Z = (0, 1), (2, 3)
    W = lambda n: [("wait", n)]
    kv = lambda *ps: [("kv", *ps)]
    kt = lambda *ps: [("kt", *ps)]
    lq = lambda *ps: [("lq", *ps)]
    K = lambda p, ls: [("k", p, ls)]
    X = lambda p, ls: [("x", p, ls)]
    C = lambda p: [("c", p, A), ("c", p, Z)]
    M = lambda m, lim=NP: [("mac", [m], lim)]
    F1 = lambda p, c0, c1: [("f1", 2 * p, 2, c0, c1, False)]
    S1 = lambda p, c0, c1: [("f1", 2 * p, 2, c0, c1, True)]
    F2 = lambda p, l0, l1: [("f2", 2 * p, 2, l0, l1)]
    FC = lambda p: lq(p + 1) + F1(p, 0, 11) + F2(p, 0, 2) + C(p + 1) + F2(p, 2, 4)
    mul = lambda v: [("set", "mul", v)]
    prog = [
        [("tables",)] + W("s0") + kt(0, 1) + K(0, A) + K(0, Z),
        W("a0") + [("hold", True), ("set", "cap1", 2.2), ("set", "capx", 1.8)]
        + kv(0) + K(1, A) + X(0, A) + X(0, Z) + M(0) + K(1, Z) + C(0)
        + W("q0") + W("g1") + [("hold", False)] + lq(0) + kv(1) + X(1, A) + X(1, Z),
        W("w1a") + [("rw1", 0, n1), ("hold", True)] + M(1) + S1(0, 0, n1 - 1) + [("c", 1, A)]
        + S1(0, n1 - 1, n1) + [("c", 1, Z)]
        + W("w1b") + [("rw1", n1, 11)] + lq(1) + S1(0, n1, n1 + 2) + [("hold", False)] + S1(0, n1 + 2, 11),
        W("g2") + mul(0.85) + [("set", "cap1", cfg["cap1"]), ("set", "capx", cfg["capx"])]
        + kt(2) + kv(2) + lq(2) + M(2, 1)
        + S1(1, 0, 2) + K(2, A) + S1(1, 2, 4) + K(2, Z) + S1(1, 4, 6) + X(2, A) + S1(1, 6, 8) + X(2, Z)
        + S1(1, 8, 11),
        W("w2") + W("g3") + mul(0.9) + [("rw2",)] + M(2) + M(3, 2) + M(4, 2) + F2(0, 0, 3) + C(2)
        + kt(3) + kv(3) + F2(0, 3, 4) + F2(1, 0, 1) + K(3, A) + K(3, Z) + F2(1, 1, 2) + X(3, A) + F2(1, 2, 3)
        + X(3, Z) + F2(1, 3, 4),
        W("g4") + mul(1.0) + kt(4) + lq(3) + M(3) + M(4, 3) + M(5, 3) + F1(2, 0, 3)
        + K(4, A) + kt(5) + F1(2, 3, 4) + K(4, Z) + F1(2, 4, 5) + K(5, A) + kt(6) + F1(2, 5, 6) + K(5, Z)
        + F1(2, 6, 7) + K(6, A) + kt(7) + F1(2, 7, 8) + K(6, Z) + kv(4, 5, 6, 7) + F1(2, 8, 9) + K(7, A)
        + F1(2, 9, 10) + K(7, Z) + F1(2, 10, 11) + C(3) + F2(2, 0, 2) + X(4, A) + F2(2, 2, 3) + X(4, Z) + X(5, A)
        + F2(2, 3, 4) + X(5, Z) + S1(3, 0, 1) + X(6, A) + S1(3, 1, 2) + X(6, Z) + S1(3, 2, 3) + X(7, A)
        + S1(3, 3, 4) + X(7, Z),
        W("q4") + mul(0.9) + lq(4) + M(4) + M(5) + M(6) + M(7)
        + S1(3, 4, 11) + F2(3, 0, 2) + C(4) + F2(3, 2, 4) + FC(4) + FC(5) + FC(6)
        + [("f1", 14, 1, 0, 11, False), ("f1", 15, 1, 0, 11, False), ("f2", 14, 1, 0, 4), ("f2", 15, 1, 0, 4)],
    ]
    return dict(dma=dma, prog=prog, cfg=cfg)


@jax.jit
def pallas_sequential_preLN__ssm_conv_h3__dense_activation_gelu__prompt_kernel(
    A_q: jax.Array,
    A_k: jax.Array,
    A_v: jax.Array,
    A_shift_k: jax.Array,
    A_ssm_k: jax.Array,
    A_ssm_D: jax.Array,
    B_x: jax.Array,
    B_w1: jax.Array,
    B_b1: jax.Array,
    B_w2: jax.Array,
    B_b2: jax.Array,
):
    plan = _plan()
    ANY = pl.BlockSpec(memory_space=pl.ANY)
    V = pltpu.VMEM
    scratch = [
        V((S, D), bf16), V((S, D), bf16), V((S, D), bf16), V((D, S), bf16),
        V((F, D), bf16), V((F, D), bf16),
        V((4, D), bf16), V((D,), bf16), V((F,), bf16), V((D,), bf16),
        V((NL, S + 16, 128), f32), V((S, D), bf16),
        V((F // 2, D), u32), V((F // 2, D), u32),
        V((128, 128), u32), V((128, 128), u32), V((128, 128), u32),
        V((NP, 3, SB, D), f32), V((NP, 3, SB, D), f32),
        V((NP, 2 * SB, D), f32), V((NP, 2 * SB, D), f32),
        V((S, D), f32), V((S, D), f32),
        V((4 * SB, F), f32), V((NL, S + 8, 128), f32), V((NL, S + 8, 128), f32),
        V((S, D), f32),
        pltpu.SMEM((1,), jnp.int32),
        pltpu.SemaphoreType.DMA((len(plan["dma"]),)), pltpu.SemaphoreType.DMA((1,)),
    ]
    out = pl.pallas_call(
        functools.partial(_kernel, plan=plan),
        grid=(len(plan["prog"]),),
        in_specs=[ANY] * 10,
        out_specs=ANY,
        out_shape=jax.ShapeDtypeStruct((S, D), bf16),
        scratch_shapes=scratch,
        compiler_params=pltpu.CompilerParams(
            dimension_semantics=("arbitrary",), vmem_limit_bytes=120 * 1024 * 1024,
            disable_semaphore_checks=True, disable_bounds_checks=True),
    )(A_q.reshape(S, D), A_k.reshape(S, D), A_v.reshape(S, D), A_shift_k.T, A_ssm_k, A_ssm_D,
      B_w1.T, B_b1, B_w2, B_b2)
    return out.reshape(1, S, D)
```
